```python
import jax
import jax.numpy as jnp

def _softmax(x, axis=-1):
    return jax.nn.softmax(x, axis=axis)
def _gelu(x):
    return jax.nn.gelu(x, approximate=True)
def _silu(x):
    return jax.nn.silu(x)
def _sigmoid(x):
    return jax.nn.sigmoid(x)
def _layernorm(x, axis=-1, eps=1e-5):
    m = jnp.mean(x, axis=axis, keepdims=True)
    v = jnp.var(x, axis=axis, keepdims=True)
    return (x - m) / jnp.sqrt(v + eps)
def _scatter_add(tgt, idx, src, axis=0):
    return tgt.at[idx].add(src)
def _segment_sum(src, seg, n):
    return jax.ops.segment_sum(src, seg, n)
class _Rng:
    def __init__(self, key):
        self._k = key
    def _next(self):
        self._k, sub = jax.random.split(self._k)
        return sub
    def normal(self, shape):
        return jax.random.normal(self._next(), shape, dtype=jnp.bfloat16)
    def randint(self, lo, hi, shape):
        return jax.random.randint(self._next(), shape, lo, hi, dtype=jnp.int32)
    def uniform(self, shape, lo=0.0, hi=1.0):
        return jax.random.uniform(self._next(), shape, jnp.bfloat16, lo, hi)
    def permutation(self, n):
        return jax.random.permutation(self._next(), n)


kernel_name = 'interleave_layers__sliding_local_dilated__softmax_full_mha__prompt'

def setup_inputs():
    _rng = _Rng(jax.random.key(int.from_bytes(__import__("os").urandom(4), "little")))
    _w = (lambda a: (lambda t: t.astype(jnp.bfloat16) if jnp.issubdtype(t.dtype, jnp.floating) else t)(jnp.asarray(a)))
    def _A_setup():
        B, S, D = 1, 2048, 1024
        return {
            "x": _w((lambda *s: _rng.normal(s) * 0.05)(B, S, D)),
            "wqkv": _w((lambda *s: _rng.normal(s) * 0.05)(D, 3 * D)),
            "wo": _w((lambda *s: _rng.normal(s) * 0.05)(D, D)),
        }
    _A_in = _A_setup()

    def _B_setup():
        B, S, D = 1, 2048, 1024
        return {
            "x": _w((lambda *s: _rng.normal(s) * 0.05)(B, S, D)),
            "wqkv": _w((lambda *s: _rng.normal(s) * 0.05)(D, 3 * D)),
            "wo": _w((lambda *s: _rng.normal(s) * 0.05)(D, D)),
        }
    _B_in = _B_setup()

    return {
        "A_x": _A_in["x"],
        "A_wqkv": _A_in["wqkv"],
        "A_wo": _A_in["wo"],
        "B_x": _B_in["x"],
        "B_wqkv": _B_in["wqkv"],
        "B_wo": _B_in["wo"],
    }

def reference(A_x, A_wqkv, A_wo, B_x, B_wqkv, B_wo):
    def _A_ref(x, wqkv, wo):
        B, S, D = x.shape
        H = 32; Dh = D // H
        W, dil = 8, 2
        qkv = (lambda x, *d: x.transpose(*d))((x @ wqkv).reshape(B, S, 3, H, Dh), 2, 0, 3, 1, 4)
        q, k, v = qkv[0], qkv[1], qkv[2]
        scale = Dh ** -0.5
        pos = jnp.arange(S)
        off = jnp.arange(W) * dil
        idx = pos[:, None] - off[None, :]
        mask = idx >= 0
        idx_c = jnp.where(mask, idx, 0).reshape(-1)
        kg = k[:, :, idx_c, :].reshape(B, H, S, W, Dh)
        vg = v[:, :, idx_c, :].reshape(B, H, S, W, Dh)
        logits = jnp.einsum("bhsd,bhswd->bhsw", q, kg) * scale
        logits = jnp.where(mask[None, None, :, :], logits, -1e9)
        attn = _softmax(logits, axis=-1)
        o = jnp.einsum("bhsw,bhswd->bhsd", attn, vg)
        return (lambda x, *d: x.transpose(*d))(o, 0, 2, 1, 3).reshape(B, S, D) @ wo

    def _B_ref(x, wqkv, wo):
        B, S, D = x.shape
        H = 32; Dh = D // H
        qkv = (lambda x, *d: x.transpose(*d))((x @ wqkv).reshape(B, S, 3, H, Dh), 2, 0, 3, 1, 4)
        q, k, v = qkv[0], qkv[1], qkv[2]
        scale = Dh ** -0.5
        scores = jnp.einsum("bhqd,bhkd->bhqk", q, k) * scale
        p = _softmax(scores, axis=-1)
        o = jnp.einsum("bhqk,bhkd->bhqd", p, v)
        return (lambda x, *d: x.transpose(*d))(o, 0, 2, 1, 3).reshape(B, S, D) @ wo

    x = A_x
    x = x + _A_ref(_layernorm(x, axis=-1), A_wqkv, A_wo)
    x = x + _B_ref(_layernorm(x, axis=-1), B_wqkv, B_wo)
    x = x + _A_ref(_layernorm(x, axis=-1), A_wqkv, A_wo)
    x = x + _B_ref(_layernorm(x, axis=-1), B_wqkv, B_wo)
    return x
```

```python
import functools
import math

import jax
import jax.numpy as jnp
from jax import lax
import jax.experimental.pallas as pl
import jax.experimental.pallas.tpu as pltpu

S = 2048
D = 1024
H = 32
DH = 32
WIN = 8
DIL = 2
HALO = 16
NT = D // 128
QB = 512
NQB = S // QB
KC = 128
QSCALE = (DH ** -0.5) * math.log2(math.e)
MASKED = -1e9 * math.log2(math.e)
F32 = jnp.float32
BF16 = jnp.bfloat16


def _layernorm(x):
    m = jnp.sum(x, axis=-1, keepdims=True) * (1.0 / D)
    c = x - m
    v = jnp.sum(c * c, axis=-1, keepdims=True) * (1.0 / D)
    return c * lax.rsqrt(v + 1e-5)


def _swap_lane_bits(tiles):
    shape = tiles[0].shape
    lane = lax.broadcasted_iota(jnp.int32, shape, 1)
    for b in range(3):
        s = 4 << b
        low = (lane & s) == 0
        new = list(tiles)
        for j in range(8):
            if j & (1 << b):
                continue
            a, c = tiles[j], tiles[j | (1 << b)]
            new[j] = jnp.where(low, a, pltpu.roll(c, s, 1))
            new[j | (1 << b)] = jnp.where(low, pltpu.roll(a, 128 - s, 1), c)
        tiles = new
    return tiles


def make(T=256, NS=2, name="k1"):
    CH = T * NS
    NCH = S // CH

    def kernel(x_hbm, wa_hbm, woa_hbm, wb_hbm, wob_hbm, out_hbm,
               xio, xres, xn, wa, woa_raw, woa, wb, wob,
               qa, ka, va, kb, qtb, vtb, sbuf, mbuf, ob, sems, osems):

        def rows(i, n):
            return pl.ds(pl.multiple_of(i * n, n), n)

        cp_wa = [pltpu.make_async_copy(wa_hbm.at[:, pl.ds(i * D, D)], wa.at[:, pl.ds(i * D, D)], sems.at[i])
                 for i in range(3)]
        cp_x = pltpu.make_async_copy(x_hbm, xio, sems.at[3])
        cp_woa = pltpu.make_async_copy(woa_hbm, woa_raw, sems.at[4])
        cp_wb = pltpu.make_async_copy(wb_hbm, wb, sems.at[5])
        cp_wob = pltpu.make_async_copy(wob_hbm, wob, sems.at[6])
        cp_x.start()
        for c in cp_wa:
            c.start()
        cp_woa.start()
        cp_wb.start()
        cp_wob.start()

        cp_x.wait()

        @pl.loop(0, S // 128)
        def _(i):
            x = xio[rows(i, 128), :].astype(F32)
            xres[rows(i, 128), :] = x
            xn[rows(i, 128), :] = _layernorm(x).astype(BF16)

        for p in range(3):
            cp_wa[p].wait()

            @pl.loop(0, D // 128)
            def _(i):
                r = rows(i, 128)
                tiles = [pltpu.bitcast(wa[r, pl.ds(p * D + j * 128, 128)], jnp.uint32) for j in range(NT)]
                tiles = _swap_lane_bits(tiles)
                for j in range(NT):
                    wa[r, pl.ds(p * D + j * 128, 128)] = pltpu.bitcast(tiles[j], BF16)

        cp_woa.wait()

        @pl.loop(0, NT)
        def _(i):
            cols = pl.ds(pl.multiple_of(i * 128, 128), 128)
            v = [pltpu.bitcast(woa_raw[pl.ds(16 * r, 16), cols], jnp.uint32) for r in range(64)]
            sub = lax.broadcasted_iota(jnp.int32, (8, 128), 0)
            for vb, s in ((4, 4), (3, 2)):
                low = (sub & s) == 0
                new = list(v)
                for r in range(64):
                    if r & (1 << vb):
                        continue
                    a, c = v[r], v[r | (1 << vb)]
                    new[r] = jnp.where(low, a, pltpu.roll(c, s, 0))
                    new[r | (1 << vb)] = jnp.where(low, pltpu.roll(a, 8 - s, 0), c)
                v = new
            for r in range(64):
                dst = (r & 0b011110) | ((r & 1) << 5) | (r >> 5)
                woa[pl.ds(16 * dst, 16), cols] = pltpu.bitcast(v[r], BF16)

        cp_wb.wait()
        cp_wob.wait()

        def qkv_a(c, j):
            xa = xn[pl.ds(pl.multiple_of(c * CH + j * T, T), T), :]
            for p, dst in enumerate((qa, ka, va)):
                y = jnp.dot(xa, wa[:, p * D:(p + 1) * D], preferred_element_type=F32)
                if p == 0:
                    y = y * QSCALE
                for t in range(NT):
                    dst[t, pl.ds(HALO + j * T, T), :] = y[:, t * 128:(t + 1) * 128]

        def attn_a(c, j):
            R = 16
            lane = lax.broadcasted_iota(jnp.int32, (R, 128), 1)
            low1 = (lane & 1) == 0
            low2 = (lane & 2) == 0
            outs = []
            for r in range(T // R):
                base = HALO + j * T + r * R
                logit = []
                for w in range(WIN):
                    acc = None
                    for t in range(NT):
                        pr = qa[t, pl.ds(base, R), :] * ka[t, pl.ds(base - DIL * w, R), :]
                        acc = pr if acc is None else acc + pr
                    acc = acc + jnp.where(low2, pltpu.roll(acc, 126, 1), pltpu.roll(acc, 2, 1))
                    acc = acc + jnp.where(low1, pltpu.roll(acc, 127, 1), pltpu.roll(acc, 1, 1))
                    if j == 0 and r * R < DIL * w:
                        pos = c * CH + r * R + lax.broadcasted_iota(jnp.int32, (R, 128), 0)
                        acc = jnp.where(pos >= DIL * w, acc, MASKED)
                    logit.append(acc)
                m = functools.reduce(jnp.maximum, logit)
                e = [jnp.exp2(l - m) for l in logit]
                inv = 1.0 / functools.reduce(jnp.add, e)
                e = [x * inv for x in e]
                o = []
                for t in range(NT):
                    acc = None
                    for w in range(WIN):
                        pr = e[w] * va[t, pl.ds(base - DIL * w, R), :]
                        acc = pr if acc is None else acc + pr
                    o.append(acc.astype(BF16))
                outs.append(jnp.concatenate(o, axis=1))
            return jnp.concatenate(outs, axis=0)

        def oproj_a(c, j, o):
            r = pl.ds(pl.multiple_of(c * CH + j * T, T), T)
            x = xres[r, :] + jnp.dot(o, woa[...], preferred_element_type=F32)
            xres[r, :] = x
            return _layernorm(x).astype(BF16)

        def qkv_b(c, j, xb):
            r = pl.ds(pl.multiple_of(c * CH + j * T, T), T)
            tok = c * CH + j * T
            q = jnp.dot(xb, wb[:, 0:D], preferred_element_type=F32) * QSCALE
            qt = q.T.astype(BF16)
            v = jnp.dot(xb, wb[:, 2 * D:3 * D], preferred_element_type=F32)
            vt = v.T.astype(BF16)
            for u in range(T // 128):
                qtb[tok // 128 + u] = qt[:, u * 128:(u + 1) * 128]
                vtb[tok // 128 + u] = vt[:, u * 128:(u + 1) * 128]
            k = jnp.dot(xb, wb[:, D:2 * D], preferred_element_type=F32).astype(BF16)
            for g in range(NT):
                kb[g, r, :] = k[:, g * 128:(g + 1) * 128]

        def proj_body(c):
            o = {}
            xb = {}
            for t in range(NS + 2):
                if t < NS:
                    qkv_a(c, t)
                    if t == 0:
                        for buf in (ka, va):
                            for g in range(NT):
                                first = jnp.broadcast_to(buf[g, pl.ds(HALO, 1), :], (HALO, 128))
                                buf[g, pl.ds(0, HALO), :] = jnp.where(c == 0, first, buf[g, pl.ds(0, HALO), :])
                    o[t] = attn_a(c, t)
                if 0 <= t - 1 < NS:
                    xb[t - 1] = oproj_a(c, t - 1, o[t - 1])
                if 0 <= t - 2 < NS:
                    qkv_b(c, t - 2, xb[t - 2])
            for buf in (ka, va):
                buf[:, pl.ds(0, HALO), :] = buf[:, pl.ds(CH, HALO), :]

        def attn_b(i, do_pv, do_scores):
            g, qb = i % NT, i // NT
            gn, qbn = (i + 1) % NT, (i + 1) // NT
            ot = []
            for u in range(4):
                if do_pv:
                    m_cur = mbuf[u]
                    acc = l = None
                if do_scores:
                    hr = pl.ds(pl.multiple_of(gn * 128 + u * DH, DH), DH)
                    qh = jnp.concatenate([qtb[qbn * (QB // 128) + a, hr, :] for a in range(QB // 128)], axis=1)
                    parts = [jnp.zeros((DH, QB), BF16)] * 4
                    parts[u] = qh
                    qm = jnp.concatenate(parts, axis=0)
                    m_next = None
                for c in range(S // KC):
                    kr = pl.ds(c * KC, KC)
                    if do_pv:
                        p = jnp.exp2(sbuf[u, kr, :].reshape(KC // 8, 8, QB) - m_cur[None])
                        lc = jnp.sum(p, axis=0)
                        l = lc if l is None else l + lc
                        vh = vtb[c, pl.ds(pl.multiple_of(g * 128 + u * DH, DH), DH), :]
                        pv = jnp.dot(vh, p.reshape(KC, QB).astype(BF16), preferred_element_type=F32)
                        acc = pv if acc is None else acc + pv
                    if do_scores:
                        s = jnp.dot(kb[gn, kr, :], qm, preferred_element_type=F32)
                        sbuf[u, kr, :] = s
                        mc = jnp.max(s.reshape(KC // 8, 8, QB), axis=0)
                        m_next = mc if m_next is None else jnp.maximum(m_next, mc)
                if do_pv:
                    ot.append(acc * (1.0 / jnp.sum(l, axis=0, keepdims=True)))
                if do_scores:
                    mbuf[u] = jnp.broadcast_to(jnp.max(m_next, axis=0, keepdims=True), (8, QB))
            if do_pv:
                ob[g, rows(qb, QB), :] = jnp.concatenate(ot, axis=0).T.astype(BF16)

        def oproj_b(c):
            for j in range(NS):
                r = pl.ds(pl.multiple_of(c * CH + j * T, T), T)
                o = jnp.concatenate([ob[g, r, :] for g in range(NT)], axis=1)
                x = xres[r, :] + jnp.dot(o, wob[...], preferred_element_type=F32)
                xres[r, :] = x
                xio[r, :] = x.astype(BF16)
                xn[r, :] = _layernorm(x).astype(BF16)

        for buf in (ka, va):
            buf[:, pl.ds(0, HALO), :] = jnp.zeros((NT, HALO, 128), F32)

        def out_copy(c):
            return pltpu.make_async_copy(xio.at[rows(c, CH)], out_hbm.at[rows(c, CH)], osems.at[c])

        @pl.loop(0, 2)
        def _(rep):
            pl.loop(0, NCH)(proj_body)
            n = NQB * NT
            attn_b(-1, False, True)
            pl.loop(0, n - 1)(lambda i: attn_b(i, True, True))
            attn_b(n - 1, True, False)

            @pl.loop(0, NCH)
            def _(c):
                oproj_b(c)

                @pl.when(rep == 1)
                def _():
                    out_copy(c).start()

        for c in range(NCH):
            out_copy(c).wait()

    def fn(A_x, A_wqkv, A_wo, B_x, B_wqkv, B_wo):
        del B_x
        hbm = pl.BlockSpec(memory_space=pltpu.HBM)
        out = pl.pallas_call(
            kernel,
            out_shape=jax.ShapeDtypeStruct((S, D), BF16),
            in_specs=[hbm] * 5,
            out_specs=hbm,
            scratch_shapes=[
                pltpu.VMEM((S, D), BF16),
                pltpu.VMEM((S, D), F32),
                pltpu.VMEM((S, D), BF16),
                pltpu.VMEM((D, 3 * D), BF16),
                pltpu.VMEM((D, D), BF16),
                pltpu.VMEM((D, D), BF16),
                pltpu.VMEM((D, 3 * D), BF16),
                pltpu.VMEM((D, D), BF16),
                pltpu.VMEM((NT, HALO + CH, 128), F32),
                pltpu.VMEM((NT, HALO + CH, 128), F32),
                pltpu.VMEM((NT, HALO + CH, 128), F32),
                pltpu.VMEM((NT, S, 128), BF16),
                pltpu.VMEM((S // 128, D, 128), BF16),
                pltpu.VMEM((S // 128, D, 128), BF16),
                pltpu.VMEM((4, S, QB), F32),
                pltpu.VMEM((4, 8, QB), F32),
                pltpu.VMEM((NT, S, 128), BF16),
                pltpu.SemaphoreType.DMA((7,)),
                pltpu.SemaphoreType.DMA((NCH,)),
            ],
            compiler_params=pltpu.CompilerParams(vmem_limit_bytes=120 * 2 ** 20),
            name=name,
        )(A_x.reshape(S, D), A_wqkv, A_wo, B_wqkv, B_wo)
        return out.reshape(1, S, D)

    fn.__name__ = name
    return jax.jit(fn)


pallas_interleave_layers__sliding_local_dilated__softmax_full_mha__prompt_kernel = make(
    name="pallas_interleave_layers__sliding_local_dilated__softmax_full_mha__prompt_kernel", T=128, NS=2)
```

```python
import contextlib
import functools
import math

import jax
import jax.numpy as jnp
from jax import lax
import jax.experimental.pallas as pl
import jax.experimental.pallas.tpu as pltpu

S = 2048
D = 1024
HD = D // 2
H = 32
DH = 32
WIN = 8
DIL = 2
HALO = 16
NT = D // 128
T = 128
HT = T // 2
NB = S // T
PR = HD // NB
QB = 512
NQB = S // QB
KC = 128
QSCALE = (DH ** -0.5) * math.log2(math.e)
MASKED = -1e9 * math.log2(math.e)
F32 = jnp.float32
BF16 = jnp.bfloat16
U32 = jnp.uint32
AQ, AK, AV, AO, BQ, BK, BV, BO = range(8)


def _pack(x):
    return pltpu.bitcast(x, U32)


def _unpack(x):
    return pltpu.bitcast(x, BF16)


def _layernorm(tiles):
    m = jnp.sum(functools.reduce(jnp.add, tiles), axis=-1, keepdims=True) * (1.0 / D)
    c = [t - m for t in tiles]
    v = jnp.sum(functools.reduce(jnp.add, [t * t for t in c]), axis=-1, keepdims=True) * (1.0 / D)
    r = lax.rsqrt(v + 1e-5)
    return [t * r for t in c]


def _swap_lane_bits(tiles):
    field = lax.broadcasted_iota(jnp.int32, tiles[0].shape, 1) >> 2
    t = [tiles[j] if j == 0 else pltpu.roll(tiles[j], 4 * j, 1) for j in range(8)]
    t = [t[-f % 8] for f in range(8)]
    for b in range(3):
        hit = (field & (1 << b)) != 0
        t = [jnp.where(hit, t[(f - (1 << b)) % 8], t[f]) for f in range(8)]
    return [t[f] if f == 0 else pltpu.roll(t[f], 128 - 4 * f, 1) for f in range(8)]


def _swap_sublane_bits(v):
    sub = lax.broadcasted_iota(jnp.int32, (8, 128), 0)
    for bit, s in ((2, 4), (1, 2)):
        low = (sub & s) == 0
        new = list(v)
        for r in range(4):
            if not r & bit:
                new[r] = jnp.where(low, v[r], pltpu.roll(v[r | bit], s, 0))
                new[r | bit] = jnp.where(low, pltpu.roll(v[r], 8 - s, 0), v[r | bit])
        v = new
    return v


def _lhs_operands(a11, a12, a21, a22):
    ops = (a11 + a22, a21 + a22, a11, a22, a11 + a12, a21 - a11, a12 - a22)
    return [a.astype(BF16) for a in ops]


def _rhs_operands(b11, b12, b21, b22):
    f11, f12, f21, f22 = (b.astype(F32) for b in (b11, b12, b21, b22))
    return [b.astype(BF16) for b in (f11 + f22, b11, f12 - f22, f21 - f11, b22, f11 + f12, f21 + f22)]


SCHED = "k0 l0:28 v0 p0:22 k1 o0 n0:18 v1 l1:26 K0 p1:22 V0 o1 n1:18 Q0 Q1 V1 K1"


def make(NS=2, NU=4, order=(0, 3, 4, 6, 2, 1, 5), name="k5", scopes=False, only=None,
         sched=SCHED, OS=4, QS=4, flags=None, gate=True, ospan=20, qspan=20, pspan=24, NQ=4, AHEAD=3):
    scope = jax.named_scope if scopes else (lambda n: contextlib.nullcontext())
    CH = T * NS
    NG = NU // 4

    def kernel(x_hbm, wa_hbm, woa_hbm, wb_hbm, wob_hbm, out_hbm,
               xio, xres, xop, top, xn, raw_a, raw_oa, raw_b, raw_ob, wq, wp,
               qa, pa, ka, va, kb, qtb, vtb, sbuf, mbuf, abuf, lbuf, xsems, wsems, osems):
        ob = qa

        def rows(i, n):
            return pl.ds(i * n if isinstance(i, int) else pl.multiple_of(i * n, n), n)

        def weight(mat):
            return wq if mat == AQ else wp.at[mat - 1]

        def now(x):
            return x

        class Pacer:
            def __init__(self, never):
                self.never = never
                self.slot = 0
                self.todo = []

            def add(self, tasks, span, delay=0):
                for k, task in enumerate(tasks):
                    self.todo.append((self.slot + delay + k * span // len(tasks), task))

            def tick(self, product):
                def after(x):
                    if not gate:
                        return x
                    p = product[:x.shape[0]]
                    return jnp.where(self.never, p if x.dtype == F32 else pltpu.bitcast(p, x.dtype), x)
                due = [t for s, t in self.todo if s <= self.slot]
                self.todo = [(s, t) for s, t in self.todo if s > self.slot]
                for task in due:
                    task(after)
                self.slot += 1

        def matmul(src, blk, mat, emit, pacer):
            for n in range(HD // 128):
                m = {}
                for r in order:
                    a = jnp.concatenate([src[r, t, rows(blk, HT // 2), :] for t in range(HD // 128)], axis=1)
                    m[r] = jnp.dot(_unpack(a), _unpack(weight(mat)[r, n]), preferred_element_type=F32)
                    pacer.tick(m[r])
                emit(n, jnp.concatenate([m[0] + m[3] - m[4] + m[6], m[3] + m[1]], axis=0))
                emit(n + HD // 128, jnp.concatenate([m[4] + m[2], m[0] + m[2] - m[1] + m[5]], axis=0))

        def stage_tasks(dst, blk, src, src_blk, make_rows=None):
            def stage(r, after):
                for t in range(HD // 128):
                    quad = [after(src[t + dt, rows(src_blk * (T // 16) + (r + dr) // 16, 16), :])
                            for dr in (0, HT) for dt in (0, 4)]
                    for k, a in enumerate(_lhs_operands(*quad)):
                        dst[k, t, rows(blk * (HT // 16) + r // 16, 8), :] = _pack(a)
            tasks = []
            for r in range(0, HT + 16, 16):
                if make_rows is not None and r < HT:
                    tasks += [functools.partial(make_rows, r + dr) for dr in (0, 8, HT, HT + 8)]
                if r > 0:
                    tasks.append(functools.partial(stage, r - 16))
            return tasks

        def norm_tasks(dst, blk, i, slot):
            def norm(r, after):
                x = [after(xres[t, rows(i * (T // 8) + r // 8, 8), :]) for t in range(NT)]
                for t, y in enumerate(_layernorm(x)):
                    xn[t, pl.ds(slot * T + r, 8), :] = y
            return stage_tasks(dst, blk, xn, slot, norm)

        raws = [(raw_a, 0), (raw_a, NT), (raw_a, 2 * NT), None, (raw_b, 0), (raw_b, NT), (raw_b, 2 * NT), (raw_ob, 0)]

        def x_copy(i):
            return pltpu.make_async_copy(x_hbm.at[rows(i, T)], xio.at[rows(i, T)], xsems.at[i])

        def copy(src, dst, idx, sem):
            return pltpu.make_async_copy(src.at[idx], dst.at[idx], wsems.at[sem])

        def aq_copy(i):
            return copy(wa_hbm, raw_a, (slice(None), rows(i, HD // NQ), pl.ds(0, D)), NB + i)

        def bo_copy():
            return copy(wob_hbm, raw_ob, (slice(None),), NB + NQ)

        def ao_tiles(i):
            return (i & 3, (i & 3) + 4)

        def step_copies(i):
            return [copy(wa_hbm, raw_a, (slice(None), rows(i, PR), pl.ds(D, 2 * D)), i),
                    copy(wb_hbm, raw_b, (slice(None), rows(i, PR)), i)] + [
                    copy(woa_hbm, raw_oa, (slice(None), i >> 2, slice(None), rows(j, 128)), i) for j in ao_tiles(i)]

        def start_step(i):
            x_copy(i + 1).start()
            for c in step_copies(i):
                c.start()

        def prep(mat, i, n, after):
            raw, tile0 = raws[mat]
            halves = []
            for k in range(2):
                tiles = [after(_pack(raw[k, rows(i, n), rows(tile0 + j, 128)])) for j in range(NT)]
                if mat in (AQ, AK, AV):
                    tiles = _swap_lane_bits(tiles)
                halves.append([_unpack(t) for t in tiles])
            for j in range(NT // 2):
                ops = _rhs_operands(halves[0][j], halves[0][j + 4], halves[1][j], halves[1][j + 4])
                for r, b in enumerate(ops):
                    weight(mat)[r, j, rows(i, n // 2), :] = _pack(b)

        def prep_ao(i, h4, after):
            b = [[_swap_sublane_bits([after(_pack(raw_oa[h4 * 4 + h, i >> 2, rows(d4, 16), rows(j, 128)]))
                                      for h in range(4)])
                  for j in ao_tiles(i)] for d4 in range(2)]
            for d in range(4):
                ops = _rhs_operands(*[_unpack(b[k][j][d]) for k in range(2) for j in range(2)])
                for r, w in enumerate(ops):
                    weight(AO)[r, i & 3, rows(d * 8 + (i >> 2) * 2 + h4, 8), :] = _pack(w)

        def load_x(i):
            x_copy(i).wait()
            for t in range(NT):
                xres[t, rows(i, T), :] = xio[rows(i, T), rows(t, 128)].astype(F32)

        x_copy(0).start()
        for i in range(NQ):
            aq_copy(i).start()
        for i in range(AHEAD):
            start_step(i)

        for buf in (ka, va):
            buf[:, pl.ds(CH, HALO), :] = jnp.zeros((NT, HALO, 128), F32)
        abuf[...] = jnp.zeros(abuf.shape, F32)
        lbuf[...] = jnp.ones(lbuf.shape, F32)

        def query_block(i, first):
            pacer = Pacer(i < 0)
            pacer.add(norm_tasks(xop, jnp.minimum(i + 1, NB - 1), jnp.minimum(i + 1, NB - 1), 0), qspan)
            if first:
                tasks = [functools.partial(prep, m, 2 * i + k, 16) for m in (AK, AV, BQ, BK, BV) for k in range(2)]
                pacer.add(tasks + [functools.partial(prep_ao, i, h4) for h4 in range(2)], pspan)

            def emit(t, y):
                qa[t, rows(i, T), :] = y * QSCALE
            matmul(top, 0, AQ, emit, pacer)

        def fetch_block(i):
            top[:, :, rows(0, HT // 2), :] = xop[:, :, rows(i, HT // 2), :]

        def proj_body(c):
            pacer = Pacer(c < 0)

            def proj_a(j, mat, dst):
                def emit(t, y):
                    dst[t, pl.ds(HALO + j * T, T), :] = y
                    if j == 0:
                        first = jnp.broadcast_to(y[0:1], (HALO, 128))
                        dst[t, pl.ds(0, HALO), :] = jnp.where(c == 0, first, dst[t, pl.ds(CH, HALO), :])
                matmul(xop, c * NS + j, mat, emit, pacer)

            def probs(j, r, after):
                lane = lax.broadcasted_iota(jnp.int32, (8, 128), 1)
                low1 = (lane & 1) == 0
                low2 = (lane & 2) == 0
                base = j * T + r
                logit = [None] * WIN
                for t in range(NT):
                    q = after(qa[t, rows(c * (CH // 8) + base // 8, 8), :])
                    for w in range(WIN):
                        pr = q * ka[t, pl.ds(HALO + base - DIL * w, 8), :]
                        logit[w] = pr if logit[w] is None else logit[w] + pr
                for w in range(WIN):
                    acc = logit[w]
                    acc = acc + jnp.where(low2, pltpu.roll(acc, 126, 1), pltpu.roll(acc, 2, 1))
                    acc = acc + jnp.where(low1, pltpu.roll(acc, 127, 1), pltpu.roll(acc, 1, 1))
                    if base < DIL * w:
                        pos = c * CH + base + lax.broadcasted_iota(jnp.int32, (8, 128), 0)
                        acc = jnp.where(pos >= DIL * w, acc, MASKED)
                    logit[w] = acc
                m = functools.reduce(jnp.maximum, logit)
                e = [jnp.exp2(l - m) for l in logit]
                inv = 1.0 / functools.reduce(jnp.add, e)
                for w in range(WIN):
                    pa[w, pl.ds(base, 8), :] = e[w] * inv

            def mix(j, r, after):
                base = j * T + r
                e = [after(pa[w, pl.ds(base, 8), :]) for w in range(WIN)]
                for t in range(NT):
                    acc = None
                    for w in range(WIN):
                        pr = e[w] * va[t, pl.ds(HALO + base - DIL * w, 8), :]
                        acc = pr if acc is None else acc + pr
                    pa[t, pl.ds(base, 8), :] = acc

            def oproj(j):
                def emit(t, y):
                    r = rows(c * NS + j, T)
                    xres[t, r, :] = xres[t, r, :] + y
                matmul(top, j, AO, emit, pacer)

            def proj_b(j, mat):
                def emit(g, y):
                    if mat == BK:
                        kb[g, rows(c * NS + j, T // 2), :] = _pack(y.astype(BF16))
                    elif mat == BQ:
                        qtb[c * NS + j, rows(g, 64), :] = _pack((y * QSCALE).astype(BF16).T)
                    else:
                        vtb[c * NS + j, rows(g, 64), :] = _pack(y.astype(BF16).T)
                matmul(top, NS + j, mat, emit, pacer)

            steps = dict(k=lambda j: proj_a(j, AK, ka), v=lambda j: proj_a(j, AV, va), o=oproj,
                         Q=lambda j: proj_b(j, BQ), K=lambda j: proj_b(j, BK), V=lambda j: proj_b(j, BV))
            tasks = dict(
                l=lambda j: [functools.partial(probs, j, r) for r in range(0, T, 8)],
                p=lambda j: stage_tasks(top, j, pa, j, functools.partial(mix, j)),
                n=lambda j: norm_tasks(top, NS + j, c * NS + j, j))
            for s in sched.split():
                if ":" in s:
                    pacer.add(tasks[s[0]](int(s[1])), int(s[3:]))
                else:
                    steps[s[0]](int(s[1]))

        GS = NT // NG
        SH = GS.bit_length() - 1

        def finish(i):
            for k in range(NG):
                ot = [abuf[u] * (1.0 / jnp.sum(lbuf[u], axis=0, keepdims=True)) for u in range(4 * k, 4 * k + 4)]
                ob[(i & (GS - 1)) * NG + k, rows(i >> SH, QB), :] = jnp.concatenate(ot, axis=0).T

        def attn_b(i, do_pv, do_scores, pacer=None):
            if do_pv:
                finish(jnp.maximum(i - 1, 0))
            for u in range(NU):
                g = (i & (GS - 1)) * NG + u // 4
                gn, qbn = ((i + 1) & (GS - 1)) * NG + u // 4, (i + 1) >> SH
                if do_pv:
                    m_cur = jnp.broadcast_to(jnp.max(mbuf[u], axis=0, keepdims=True), (8, QB))
                    l = None
                if do_scores:
                    hr = rows(gn * 4 + u % 4, DH // 2)
                    qh = jnp.concatenate([qtb[qbn * (QB // 128) + a, hr, :] for a in range(QB // 128)], axis=1)
                    parts = [jnp.zeros((DH, QB), BF16)] * 4
                    parts[u % 4] = _unpack(qh)
                    qm = jnp.concatenate(parts, axis=0)
                    m_next = None
                for c in range(S // KC):
                    kr = pl.ds(c * KC, KC)
                    if do_pv:
                        sc = sbuf[u, kr, :].reshape(KC // 8, 8, QB)
                    if do_scores:
                        s = jnp.dot(_unpack(kb[gn, rows(c, KC // 2), :]), qm, preferred_element_type=F32)
                        sbuf[u, kr, :] = s
                        if pacer is not None:
                            pacer.tick(s[:, :128])
                        s = s.reshape(KC // 8, 8, QB)
                        for r in range(KC // 8):
                            m_next = s[r] if m_next is None else jnp.maximum(m_next, s[r])
                    if do_pv:
                        p = jnp.exp2(sc - m_cur[None])
                        for r in reversed(range(KC // 8)):
                            l = p[r] if l is None else l + p[r]
                        vh = _unpack(vtb[c, rows(g * 4 + u % 4, DH // 2), :])
                        pv = jnp.dot(vh, p.reshape(KC, QB).astype(BF16), preferred_element_type=F32)
                        abuf[u] = pv if c == 0 else abuf[u] + pv
                if do_pv:
                    lbuf[u] = l
                if do_scores:
                    mbuf[u] = m_next

        def oproj_b(c):
            pacer = Pacer(c < 0)
            for task in stage_tasks(top, 0, ob, c * OS):
                task(now)
            for j in range(OS):
                i = c * OS + j
                if j + 1 < OS:
                    pacer.add(stage_tasks(top, j + 1, ob, i + 1), ospan)

                def emit(t, y):
                    x = xres[t, rows(i, T), :] + y
                    xres[t, rows(i, T), :] = x
                    xio[rows(i, T), rows(t, 128)] = x.astype(BF16)
                matmul(top, j, BO, emit, pacer)

        def out_copy(c):
            return pltpu.make_async_copy(xio.at[rows(c, OS * T)], out_hbm.at[rows(c, OS * T)], osems.at[c])

        with scope("start"):
            load_x(0)

        @pl.loop(0, 2)
        def _(rep):
            with scope("norm0"):
                for task in norm_tasks(xop, 0, 0, 0):
                    task(now)

            @pl.when(rep == 0)
            def _():
                with scope("prepq"):
                    @pl.loop(0, NQ)
                    def _(i):
                        aq_copy(i).wait()
                        for k in range(2):
                            prep(AQ, 2 * i + k, HD // NQ // 2, now)

                with scope("q0"):
                    @pl.loop(0, NB)
                    def _(i):
                        pl.when(i + AHEAD < NB - 1)(lambda: start_step(i + AHEAD))

                        @pl.when(i + AHEAD == NB - 1)
                        def _():
                            for c in step_copies(NB - 1) + [bo_copy()]:
                                c.start()

                        pl.when(i + 1 < NB)(lambda: load_x(i + 1))
                        fetch_block(i)
                        for c in step_copies(i):
                            c.wait()
                        query_block(i, True)

            @pl.when(rep == 1)
            def _():
                with scope("q1"):
                    @pl.loop(0, NB)
                    def _(i):
                        fetch_block(i)
                        query_block(i, False)

            with scope("proj"):
                pl.loop(0, S // CH)(proj_body)

            @pl.when(rep == 0)
            def _():
                bo_copy().wait()

            n = NQB * GS
            if only is None:
                with scope("pro"):
                    pacer = Pacer(rep < 0)
                    pacer.add([functools.partial(prep, BO, i, 16) for i in range(HD // 16)], 60)
                    attn_b(-1, False, True, pacer)
                with scope("attn"):
                    pl.loop(0, n - 1)(lambda i: attn_b(i, True, True))
                with scope("epi"):
                    attn_b(n - 1, True, False)
                    finish(n - 1)
            else:
                ob[0, :, :] = _unpack(kb[rep]).astype(F32)
                ob[1, pl.ds(0, D), :] = _unpack(qtb[rep]).astype(F32)
                ob[2, pl.ds(0, D), :] = _unpack(vtb[rep]).astype(F32)

            @pl.loop(0, NB // OS)
            def _(c):
                with scope("oproj"):
                    oproj_b(c)

                @pl.when(rep == 1)
                def _():
                    out_copy(c).start()

        with scope("end"):
            for c in range(NB // OS):
                out_copy(c).wait()

    def fn(A_x, A_wqkv, A_wo, B_x, B_wqkv, B_wo):
        del B_x
        hbm = pl.BlockSpec(memory_space=pltpu.HBM)
        out = pl.pallas_call(
            kernel,
            out_shape=jax.ShapeDtypeStruct((S, D), BF16),
            in_specs=[hbm] * 5,
            out_specs=hbm,
            scratch_shapes=[
                pltpu.VMEM((S, D), BF16),
                pltpu.VMEM((NT, S, 128), F32),
                pltpu.VMEM((7, 4, S // 4, 128), U32),
                pltpu.VMEM((7, 4, max(2 * NS, OS) * HT // 2, 128), U32),
                pltpu.VMEM((NT, NS * T, 128), F32),
                pltpu.VMEM((2, HD, 3 * D), BF16),
                pltpu.VMEM((8, 4, DH, D), BF16),
                pltpu.VMEM((2, HD, 3 * D), BF16),
                pltpu.VMEM((2, HD, D), BF16),
                pltpu.VMEM((7, 4, HD // 2, 128), U32),
                pltpu.VMEM((7, 7, 4, HD // 2, 128), U32),
                pltpu.VMEM((NT, S, 128), F32),
                pltpu.VMEM((NT, CH, 128), F32),
                pltpu.VMEM((NT, HALO + CH, 128), F32),
                pltpu.VMEM((NT, HALO + CH, 128), F32),
                pltpu.VMEM((NT, S // 2, 128), U32),
                pltpu.VMEM((S // 128, D // 2, 128), U32),
                pltpu.VMEM((S // 128, D // 2, 128), U32),
                pltpu.VMEM((NU, S, QB), F32),
                pltpu.VMEM((NU, 8, QB), F32),
                pltpu.VMEM((NU, DH, QB), F32),
                pltpu.VMEM((NU, 8, QB), F32),
                pltpu.SemaphoreType.DMA((NB,)),
                pltpu.SemaphoreType.DMA((NB + NQ + 1,)),
                pltpu.SemaphoreType.DMA((NB // OS,)),
            ],
            compiler_params=pltpu.CompilerParams(vmem_limit_bytes=126 * 2 ** 20, flags=flags),
            name=name,
        )(A_x.reshape(S, D), A_wqkv.reshape(2, HD, 3 * D), A_wo.reshape(8, 4, DH, D),
          B_wqkv.reshape(2, HD, 3 * D), B_wo.reshape(2, HD, D))
        return out.reshape(1, S, D)

    fn.__name__ = name
    return jax.jit(fn)


pallas_interleave_layers__sliding_local_dilated__softmax_full_mha__prompt_kernel = make(
    name="pallas_interleave_layers__sliding_local_dilated__softmax_full_mha__prompt_kernel", )
```

```python
import contextlib
import functools
import math

import jax
import jax.numpy as jnp
from jax import lax
import jax.experimental.pallas as pl
import jax.experimental.pallas.tpu as pltpu

S = 2048
D = 1024
DH = 32
WIN, DIL = 8, 2
HALO = 16
NT = D // 128
HT = 64
T = 2 * HT
NB = S // T
QB = 512
QT = QB // 128
NQB = S // QB
KC = 128
NU = 4
QSCALE = (DH ** -0.5) * math.log2(math.e)
MASKED = -1e9 * math.log2(math.e)
F32, BF16, U32 = jnp.float32, jnp.bfloat16, jnp.uint32
AQ, AK, AV, AO, BQ, BK, BV, BO = range(8)

LHS = (((1, 0, 0), (1, 1, 1)), ((1, 1, 0), (1, 1, 1)), ((1, 0, 0),), ((1, 1, 1),),
       ((1, 0, 0), (1, 0, 1)), ((1, 1, 0), (-1, 0, 0)), ((1, 0, 1), (-1, 1, 1)))
RHS = (((1, 0, 0), (1, 1, 1)), ((1, 0, 0),), ((1, 0, 1), (-1, 1, 1)), ((1, 1, 0), (-1, 0, 0)),
       ((1, 1, 1),), ((1, 0, 0), (1, 0, 1)), ((1, 1, 0), (1, 1, 1)))
ORDER = (0, 3, 4, 6, 2, 1, 5)


def _combine(m):
    return ((m[0] + m[3] - m[4] + m[6], m[4] + m[2]), (m[3] + m[1], m[0] + m[2] - m[1] + m[5]))


def _signed_sum(terms, block):
    total = block(*terms[0][1:])
    for sign, i, j in terms[1:]:
        total = total + block(i, j) if sign > 0 else total - block(i, j)
    return total


def _operands(table, block):
    grid = {(i, j): block(i, j) for i in range(2) for j in range(2)}
    return [_pack(_signed_sum(terms, lambda i, j: grid[i, j]).astype(BF16)) for terms in table]


def _operands2(table, block, r):
    return _operands(table, lambda i, j: _signed_sum(table[r], lambda a, b: block(2 * a + i, 2 * b + j)))


def _pack(x):
    return pltpu.bitcast(x, U32)


def _unpack(x):
    return pltpu.bitcast(x, BF16)


def _now(x):
    return x


def _rows(i, n):
    return pl.ds(i * n if isinstance(i, int) else pl.multiple_of(i * n, n), n)


def _bit_clear(shape, axis, bit):
    return (lax.broadcasted_iota(jnp.int32, shape, axis) & bit) == 0


def _swap_lane_bits(tiles):
    last = tiles[0].ndim - 1
    t = [tiles[j] if j == 0 else pltpu.roll(tiles[j], 4 * j, last) for j in range(8)]
    t = [t[-f % 8] for f in range(8)]
    for b in range(3):
        clear = _bit_clear(t[0].shape, last, 4 << b)
        t = [lax.select(clear, t[f], t[(f - (1 << b)) % 8]) for f in range(8)]
    return [t[f] if f == 0 else pltpu.roll(t[f], 128 - 4 * f, last) for f in range(8)]


def _swap_sublane_bits(v):
    for bit, s in ((2, 4), (1, 2)):
        clear = _bit_clear((8, 128), 0, s)
        new = list(v)
        for r in range(4):
            if not r & bit:
                new[r] = lax.select(clear, v[r], pltpu.roll(v[r | bit], s, 0))
                new[r | bit] = lax.select(clear, pltpu.roll(v[r], 8 - s, 0), v[r | bit])
        v = new
    return v


class _Pacer:
    def __init__(self, never):
        self.never = never
        self.masks = {}
        self.slot = 0
        self.todo = []

    def add(self, tasks, span, delay=0):
        for k, task in enumerate(tasks):
            self.todo.append((self.slot + delay + k * span // len(tasks), task))

    def _run(self, after):
        due = [t for s, t in self.todo if s < self.slot]
        self.todo = [(s, t) for s, t in self.todo if s >= self.slot]
        for task in due:
            task(after)

    def overdue(self):
        self._run(_now)

    def tick(self, result, row=0):
        seen = {}

        def after(x):
            if x.shape not in self.masks:
                self.masks[x.shape] = jnp.broadcast_to(self.never, x.shape)
            if (x.shape, x.dtype) not in seen:
                r = result[row:row + x.shape[-2], :128]
                r = r if x.dtype == F32 else pltpu.bitcast(r, x.dtype)
                seen[x.shape, x.dtype] = jnp.broadcast_to(r, x.shape)
            return lax.select(self.masks[x.shape], seen[x.shape, x.dtype], x)
        self.slot += 1
        self._run(after)


SCHED = ("w0:28 k0 l0:26 k1 l1:26 k2 l2:26 k3 l3:26 v0 s0:14 s1:14:14 w1:28 v1 s2:14 s3:14:14 p0:40 "
         "v2 p1:36:12 v3 p2:30:16 o0 p3:30:18 o1 w2:20:18 o2 w3:20:6 o3")


def make(name="k10", scopes=False, only=None, sched=SCHED, QS=4, flags=None, ospan=(26, 66), qspan=22, pspan=50,
         NQ=4, AHEAD=2, NV=6, NV0=0, DS=4, lead=12, epre=12, bspan=250, efrac=190):
    scope = jax.named_scope if scopes else (lambda n: contextlib.nullcontext())
    NS = 4
    CH = T * NS
    NP = NB // 2
    W2, W4 = D // 2, D // 4

    def kernel(x_hbm, wa_hbm, woa_hbm, wb_hbm, wob_hbm, out_hbm,
               xio, xres, xop, top, bop, xn, raw_b, raw_ob, wq, wa, wb,
               qa, pa, ka, va, kb, qtb, vtb, mbuf, abuf, lbuf, linv, qf, kf, xsems, wsems, osems):

        def weight(mat):
            return wq if mat == AQ else wa.at[mat - AK] if mat < BQ else wb.at[mat - BQ]

        def matmul(src, mat, emit, pacer):
            for n in range(NT // 2):
                m = {}
                for r in ORDER:
                    m[r] = jnp.dot(_unpack(src[r]), _unpack(weight(mat)[r, n]), preferred_element_type=F32)
                    pacer.tick(m[r])
                c = _combine(m)
                for j in range(2):
                    emit(n + j * (NT // 2), jnp.concatenate([c[0][j], c[1][j]], axis=0))

        def products2(src, mat, emit, pacer):
            for n in range(NT // 4):
                outer = {}
                for r1 in ORDER:
                    m = {}
                    for r2 in ORDER:
                        m[r2] = jnp.dot(_unpack(src[7 * r1 + r2]), _unpack(weight(mat)[7 * r1 + r2, n]),
                                        preferred_element_type=F32)
                        pacer.tick(m[r2])
                        yield
                    outer[r1] = _combine(m)
                c = [[_combine({r: outer[r][i][j] for r in ORDER}) for j in range(2)] for i in range(2)]
                for j in range(4):
                    emit(n + j * (NT // 4),
                         jnp.concatenate([c[i % 2][j % 2][i // 2][j // 2] for i in range(4)], axis=0))

        def stage_tasks(dsts, g, src, make_rows):
            def block(r, t, after):
                return lambda i, j: after(src[t + j * (NT // g), pl.ds(i * HT + r, 16), :])

            def store(k, r, t, ops):
                ops = jnp.stack(ops)
                for dst in dsts:
                    dst[pl.ds(k, 7), _rows(r // 16, 8), _rows(t, 128)] = ops

            def stage(r, after):
                for t in range(NT // g):
                    store(0, r, t, _operands(LHS, block(r, t, after)))

            def stage2(r, t, r1, after):
                store(7 * r1, r, t, _operands2(LHS, block(r, t, after), r1))

            if make_rows is None:
                return [functools.partial(stage2, r, t, r1)
                        for r1 in ORDER for t in range(NT // g) for r in range(0, HT, 16)]
            tasks = []
            for r in range(0, HT + 16, 16):
                if r < HT:
                    tasks += [functools.partial(make_rows, i * HT + r + dr) for i in range(g) for dr in (0, 8)]
                if r > 0 and g == 2:
                    tasks.append(functools.partial(stage, r - 16))
                elif r > 0:
                    tasks += [functools.partial(stage2, r - 16, t, r1) for t in range(NT // g) for r1 in ORDER]
            return tasks

        def norm_tasks(dsts, g, i, slot=0):
            x = xres.at[:, _rows(i, g * HT)]
            y = xn.at[:, _rows(slot, g * HT)]
            mean = {}

            def means(r0, after):
                for r in (r0, r0 + 8, r0 + HT, r0 + HT + 8):
                    total = after(jnp.sum(x[:, pl.ds(r, 8), :], axis=0))
                    mean[r] = jnp.sum(total, axis=-1, keepdims=True) * (1.0 / D)

            def norm(r, after):
                c = x[:, pl.ds(r, 8), :] - after(jnp.broadcast_to(mean[r], (8, 128)))[None]
                var = jnp.sum(jnp.sum(c * c, axis=0), axis=-1, keepdims=True) * (1.0 / D)
                y[:, pl.ds(r, 8), :] = c * lax.rsqrt(var + 1e-5)[None]
            return ([functools.partial(means, k + r) for r in range(0, HT, 16) for k in range(0, g * HT, T)]
                    + stage_tasks(dsts, g, y, norm))

        def prep_a(mat, raw, i, n, after):
            w = _swap_lane_bits([after(_pack(raw[:, _rows(i, n), _rows(mat * NT + j, 128)])) for j in range(NT)])
            for t in range(NT // 2):
                weight(mat)[:, t, _rows(i, n // 2), :] = jnp.stack(
                    _operands(RHS, lambda k, j: _unpack(w[t + j * (NT // 2)][k]).astype(F32)))

        def prep_b_tasks(mat, i):
            raw, tile0 = (raw_ob, 0) if mat == BO else (raw_b, (mat - BQ) * NT)
            src, dst = _rows(i, 16), _rows(i, 8)

            def task(t, r1, after):
                def block(k, j):
                    return _unpack(after(_pack(raw[k, src, _rows(tile0 + t + j * (NT // 4), 128)]))).astype(F32)
                weight(mat)[pl.ds(7 * r1, 7), t, dst, :] = jnp.stack(_operands2(RHS, block, r1))
            return [functools.partial(task, t, r1) for t in range(NT // 4) for r1 in ORDER]

        def first_norm():
            for task in norm_tasks((top.at[0], xop.at[0]), 2, 0):
                task(_now)

        def query_body(c, n, pacer):
            for j in range(n):
                nxt = c * n + j + 1
                if j == n - 1:
                    nxt = jnp.minimum(nxt, NB - 1)
                pacer.add(norm_tasks((top.at[(j + 1) % n], xop.at[nxt]), 2, nxt, j % 2), qspan)
                r = _rows(c * n + j, T)

                def emit(t, y):
                    qa[t, r, :] = y * QSCALE
                matmul(top.at[j], AQ, emit, pacer)

        def window_body(c):
            pacer = _Pacer(c < 0)
            q_chunk = qa.at[:, _rows(c, CH)]
            x_chunk = xres.at[:, _rows(c, CH)]
            clear = {s: _bit_clear((WIN, 8, 128), 2, s) for s in (1, 2)}

            def project(mat, dst, j):
                def emit(t, y):
                    dst[t, pl.ds(HALO + j * T, T), :] = y
                    if j == 0:
                        first = jnp.broadcast_to(y[0:1], (HALO, 128))
                        dst[t, pl.ds(0, HALO), :] = jnp.where(c == 0, first, dst[t, pl.ds(CH, HALO), :])
                matmul(xop.at[c * NS + j], mat, emit, pacer)

            def pair_sum(x, s):
                return x + lax.select(clear[s], pltpu.roll(x, 128 - s, 2), pltpu.roll(x, s, 2))

            def logits(r, after):
                q = after(q_chunk[:, pl.ds(r, 8), :])
                x = jnp.stack([jnp.sum(q * ka[:, pl.ds(HALO + r - DIL * w, 8), :], axis=0) for w in range(WIN)])
                pa[:, pl.ds(r, 8), :] = pair_sum(x, 2)

            def probs(r, after):
                x = pair_sum(after(pa[:, pl.ds(r, 8), :]), 1)
                if r < DIL * (WIN - 1):
                    pos = c * CH + r + lax.broadcasted_iota(jnp.int32, x.shape, 1)
                    x = jnp.where(pos >= DIL * lax.broadcasted_iota(jnp.int32, x.shape, 0), x, MASKED)
                e = jnp.exp2(x - jnp.max(x, axis=0, keepdims=True))
                pa[:, pl.ds(r, 8), :] = e * (1.0 / jnp.sum(e, axis=0, keepdims=True))

            def mix(r, after):
                e = after(pa[:, pl.ds(r, 8), :])
                pa[:, pl.ds(r, 8), :] = functools.reduce(
                    jnp.add, [e[w:w + 1] * va[:, pl.ds(HALO + r - DIL * w, 8), :] for w in range(WIN)])

            def project_out(j):
                def emit(t, y):
                    x_chunk[t, _rows(j, T), :] = x_chunk[t, _rows(j, T), :] + y
                matmul(top.at[j], AO, emit, pacer)

            order = [r + dr for r in range(0, HT, 16) for dr in (0, 8, HT, HT + 8)]
            matmuls = dict(k=functools.partial(project, AK, ka), v=functools.partial(project, AV, va), o=project_out)
            tasks = dict(
                l=lambda j: [functools.partial(logits, j * T + r) for r in order],
                s=lambda j: [functools.partial(probs, j * T + r) for r in order],
                p=lambda j: stage_tasks((top.at[j],), 2, pa.at[:, _rows(j, T)],
                                        lambda r, after: mix(j * T + r, after)),
                w=lambda k: [t for m in (BQ, BK, BV) for t in prep_b_tasks(m, c * NS + k)])
            for s in sched.split():
                if ":" in s:
                    pacer.add(tasks[s[0]](int(s[1])), *map(int, s[3:].split(":")))
                else:
                    matmuls[s[0]](int(s[1]))

        def qkv_body(c):
            pacer = _Pacer(c < 0)
            for j in range(2):
                i = 2 * c + j
                pacer.add(norm_tasks((bop.at[1 - j],), 4, jnp.minimum(i + 1, NB // 2 - 1)), bspan)
                for mat in (BQ, BV, BK):
                    def emit(g, y):
                        if mat == BK:
                            kb[g, _rows(i, T), :] = _pack(y.astype(BF16))
                            return
                        y = (y * QSCALE if mat == BQ else y).astype(BF16)
                        for k in range(2):
                            (qtb if mat == BQ else vtb)[2 * i + k, _rows(g, 64), :] = _pack(y[k * T:(k + 1) * T].T)
                    for _ in products2(bop.at[j], mat, emit, pacer):
                        pass

        def out_t(qb, a, head, n=1):
            return qa.at[qb * (QT // 2) + a // 2, _rows((a % 2) * (D // DH // n) + head, n * DH)]

        def attend(sbuf, i, pacer, nv, do_pv, do_scores, between=None):
            on_vpu = [k * (S // KC) // nv for k in range(nv)]
            m_next = [None] * NU
            part = {}

            def keep(u, r, s):
                sbuf[u, pl.ds(r, s.shape[0]), :] = s
                m = jnp.max(s.reshape(-1, 8, QB), axis=0)
                m_next[u] = m if m_next[u] is None else jnp.maximum(m_next[u], m)

            def vpu_scores(u, r, d0, after):
                k = after(kf[_rows(r, 8), :])
                for d in range(d0, d0 + DS):
                    kd = jnp.broadcast_to(k[:, u * DH + d:u * DH + d + 1], (QT, 8, 128))
                    pr = kd * jnp.broadcast_to(qf[u, :, pl.ds(d, 1), pl.ds(0, 128)], (QT, 8, 128))
                    part[u] = pr if d == 0 else part[u] + pr
                if d0 + DS == DH:
                    keep(u, on_vpu[r // 2] * KC + (r % 2) * 8,
                         jnp.concatenate([part[u][a] for a in range(QT)], axis=1))

            if do_scores:
                gn, qbn = (i + 1) & (NT - 1), (i + 1) >> 3
                qm = []
                for u in range(NU):
                    qh = _unpack(qtb[_rows(qbn, QT), _rows(gn * NU + u, DH // 2), :])
                    if nv:
                        qf[u, :, :, pl.ds(0, 128)] = qh.astype(F32)
                    parts = [jnp.zeros((DH, QB), BF16)] * NU
                    parts[u] = jnp.concatenate([qh[a] for a in range(QT)], axis=1)
                    qm.append(jnp.concatenate(parts, axis=0))
                for j, c in enumerate(on_vpu):
                    kf[_rows(j, 16), :] = _unpack(kb[gn, _rows(c * (KC // 16), 8), :]).astype(F32)
                pacer.add([functools.partial(vpu_scores, u, r, d0)
                           for u in range(NU) for r in range(2 * nv) for d0 in range(0, DH, DS)],
                          NU * (S - 16 * nv) // 8, -lead)
            for u in range(NU):
                if do_pv:
                    head = (i & (NT - 1)) * NU + u
                    v_rows = _rows(head, DH // 2)
                    m_cur = jnp.broadcast_to(jnp.max(mbuf[u], axis=0, keepdims=True), (8, QB))[None]
                    l = None
                for c in range(S // KC):
                    if do_pv:
                        sc = sbuf[u, _rows(c, KC), :].reshape(KC // 8, 8, QB)
                    if do_scores:
                        pacer.overdue()
                        skip = 16 if c in on_vpu else 0
                        keys = _unpack(kb[gn, pl.ds((c * KC + skip) // 2, (KC - skip) // 2), :])
                        s = jnp.dot(keys, qm[u], preferred_element_type=F32)
                        keep(u, c * KC + skip, s)
                        for r in range(0, KC - skip, 8):
                            pacer.tick(s, r)
                    if do_pv:
                        p = jnp.exp2(sc - m_cur).reshape(KC, QB)
                        for r in reversed(range(0, KC, 8)):
                            l = p[r:r + 8] if l is None else l + p[r:r + 8]
                        pv = jnp.dot(_unpack(vtb[c, v_rows, :]), p.astype(BF16), preferred_element_type=F32)
                        acc = pv if c == 0 else abuf[u] + pv
                        if c + 1 < S // KC:
                            abuf[u] = acc
                    if between is not None:
                        between()
                if do_pv:
                    for a in range(QT):
                        lbuf[(i >> 3) * QT + a, _rows(head, 8), :] = l[:, a * 128:(a + 1) * 128]
                        out_t(i >> 3, a, head)[...] = acc[:, a * 128:(a + 1) * 128]
                if do_scores:
                    mbuf[u] = m_next[u]

        def out_stage_tasks(qb, j):
            def invert(a, after):
                l = [lbuf[qb * QT + 2 * j + a, pl.ds(k, D // DH, stride=8), :] for k in range(8)]
                linv[:, _rows(a, 128)] = 1.0 / after(functools.reduce(jnp.add, l))

            def normalise(a, g, after):
                inv = after(jnp.stack([jnp.broadcast_to(linv[pl.ds(NU * g + u, 1), _rows(a, 128)], (8, 128))
                                       for u in range(NU)]))
                o = out_t(qb, 2 * j + a, g, NU)[...].reshape(NU, DH // 8, 8, 128) * inv[:, None]
                xn[g, _rows(a, T), :] = o.reshape(128, 128).T
            return ([functools.partial(invert, a) for a in range(2)]
                    + [functools.partial(normalise, a, g) for t in range(2) for g in range(t, NT, 2) for a in range(2)],
                    stage_tasks((bop.at[j],), 4, xn, None))

        def out_products(qb, nxt, pacer):
            for j in range(2):
                first, second = out_stage_tasks(nxt, 0) if j else out_stage_tasks(qb, 1)
                pacer.add(first, ospan[0])
                pacer.add(second, ospan[1], ospan[0])
                r = _rows(2 * qb + j, 2 * T)

                def emit(t, y):
                    x = xres[t, r, :] + y
                    xres[t, r, :] = x
                    xio[r, _rows(t, 128)] = x.astype(BF16)
                yield from products2(bop.at[j], BO, emit, pacer)

        def attention(rep, sbuf):
            n = NQB * NT
            if only is None:
                with scope("pro"):
                    pacer = _Pacer(rep < 0)
                    pacer.add([t for i in range(W4 // 16) for t in prep_b_tasks(BO, i)], 230 * NU)
                    attend(sbuf, -1, pacer, NV0, False, True)
                with scope("attn"):
                    pl.loop(0, n - 1)(lambda i: attend(sbuf, i, _Pacer(i < 0), NV, True, True))
            else:
                qa[0, :, :] = _unpack(kb[rep]).astype(F32)
                qa[1, pl.ds(0, D), :] = _unpack(qtb[rep]).astype(F32)
                qa[2, pl.ds(0, D), :] = _unpack(vtb[rep]).astype(F32)
            with scope("epi"):
                for tasks in out_stage_tasks(0, 0):
                    for task in tasks:
                        task(_now)
                out = out_products(0, 1, _Pacer(rep < 0))
                total, count = NU * (S // KC), [0, 0]

                def between():
                    count[0] += 1
                    while count[1] * (total - epre) < (count[0] - epre) * efrac:
                        next(out)
                        count[1] += 1
                attend(sbuf, n - 1, None, 0, True, False, between)
                for _ in out:
                    pass

        def x_copy(i):
            return pltpu.make_async_copy(x_hbm.at[_rows(i, T)], xio.at[_rows(i, T)], xsems.at[i])

        def copy(src, dst, idx, sem):
            return pltpu.make_async_copy(src.at[idx], dst.at[idx], wsems.at[sem])

        def b_copy(c):
            return copy(wb_hbm, raw_b, (slice(None), _rows(c, W4 // (S // CH))), NP + NQ + c)

        def bo_copy():
            return copy(wob_hbm, raw_ob, (slice(None),), NP + NQ + S // CH)

        def out_copy(c):
            return pltpu.make_async_copy(xio.at[_rows(c, QB)], out_hbm.at[_rows(c, QB)], osems.at[c])

        def load_x(i):
            x_copy(i).wait()
            for t in range(NT):
                xres[t, _rows(i, T), :] = xio[_rows(i, T), _rows(t, 128)].astype(F32)

        def start_up(raw_a, raw_oa):
            PR = W2 // NP

            def aq_copy(i):
                return copy(wa_hbm, raw_a, (slice(None), _rows(i, W2 // NQ), pl.ds(0, D)), NP + i)

            def ao_tiles(i):
                return (i & 3, (i & 3) + 4)

            def step_copies(i):
                return [copy(wa_hbm, raw_a, (slice(None), _rows(i, PR), pl.ds(D, 2 * D)), i)] + [
                    copy(woa_hbm, raw_oa, (slice(None), i >> 2, slice(None), _rows(j, 128)), i) for j in ao_tiles(i)]

            def start_step(i, last=False):
                x_copy(2 * i + 1).start()
                if not last:
                    x_copy(2 * i + 2).start()
                for c in step_copies(i):
                    c.start()
                if last:
                    for c in range(S // CH):
                        b_copy(c).start()
                    bo_copy().start()

            def prep_ao(i, h4, h0, after):
                b = [[_swap_sublane_bits(
                    [after(_pack(raw_oa[h4 * 4 + h, i >> 2, _rows(2 * h0 + d4, 16), _rows(j, 128)])) for h in range(4)])
                    for j in ao_tiles(i)] for d4 in range(2)]
                for d in range(4):
                    weight(AO)[:, i & 3, _rows(d * 8 + (i >> 2) * 4 + h0 * 2 + h4, 8), :] = jnp.stack(
                        _operands(RHS, lambda k, j: _unpack(b[k][j][d]).astype(F32)))

            x_copy(0).start()
            for i in range(NQ):
                aq_copy(i).start()
            for i in range(AHEAD):
                start_step(i)
            for buf in (ka, va):
                buf[:, pl.ds(CH, HALO), :] = jnp.zeros((NT, HALO, 128), F32)
            with scope("start"):
                load_x(0)
                first_norm()

            with scope("prepq"):
                @pl.loop(0, NQ)
                def _(i):
                    aq_copy(i).wait()
                    prep_a(AQ, raw_a, i, W2 // NQ, _now)

            with scope("q0"):
                @pl.loop(0, NP)
                def _(i):
                    pl.when(i + AHEAD < NP - 1)(lambda: start_step(i + AHEAD))
                    pl.when(i + AHEAD == NP - 1)(lambda: start_step(NP - 1, True))
                    load_x(2 * i + 1)
                    pl.when(i < NP - 1)(lambda: load_x(2 * i + 2))
                    for c in step_copies(i):
                        c.wait()
                    pacer = _Pacer(i < 0)
                    tasks = []
                    for k in range(PR // 16):
                        tasks += [functools.partial(prep_a, m, raw_a, i * (PR // 16) + k, 16) for m in (AK, AV)]
                        tasks.append(functools.partial(prep_ao, i, k // 2, k % 2))
                    pacer.add(tasks, pspan, -2)
                    pacer.overdue()
                    query_body(i, 2, pacer)

        pl.run_scoped(start_up, pltpu.VMEM((2, W2, 3 * D), BF16), pltpu.VMEM((8, 2, 2 * DH, D), BF16))

        @pl.loop(0, 2)
        def _(rep):
            with scope("proja"):
                @pl.loop(0, S // CH)
                def _(c):
                    pl.when(rep == 0)(lambda: b_copy(c).wait())
                    if only != 3:
                        window_body(c)
            pl.when(rep == 0)(lambda: bo_copy().wait())
            if only == 2:
                xio[pl.ds(0, 256), pl.ds(0, 128)] = _unpack(wb[rep, rep, 0]) + xres[rep, pl.ds(0, 256)].astype(BF16)
                return
            with scope("normb"):
                for task in norm_tasks((bop.at[0],), 4, 0):
                    task(_now)
            with scope("projb"):
                if only is None:
                    pl.loop(0, NB // 4)(qkv_body)
            pl.run_scoped(functools.partial(attention, rep), pltpu.VMEM((NU, S, QB), F32))
            pl.when(rep == 1)(lambda: out_copy(0).start())

            @pl.loop(1, NQB)
            def _(c):
                with scope("oproj"):
                    for _ in out_products(c, jnp.minimum(c + 1, NQB - 1), _Pacer(c < 0)):
                        pass
                pl.when(rep == 1)(lambda: out_copy(c).start())

            @pl.when(rep == 0)
            def _():
                with scope("q1"):
                    first_norm()
                    pl.loop(0, NB // QS)(lambda c: query_body(c, QS, _Pacer(c < 0)))

        with scope("end"):
            for c in range(NQB):
                if only == 2:
                    out_copy(c).start()
                out_copy(c).wait()

    def fn(A_x, A_wqkv, A_wo, B_x, B_wqkv, B_wo):
        del B_x
        hbm = pl.BlockSpec(memory_space=pltpu.HBM)
        out = pl.pallas_call(
            kernel,
            out_shape=jax.ShapeDtypeStruct((S, D), BF16),
            in_specs=[hbm] * 5,
            out_specs=hbm,
            scratch_shapes=[
                pltpu.VMEM((S, D), BF16),
                pltpu.VMEM((NT, S, 128), F32),
                pltpu.VMEM((NB, 7, HT // 2, W2), U32),
                pltpu.VMEM((max(NS, QS), 7, HT // 2, W2), U32),
                pltpu.VMEM((2, 49, HT // 2, W4), U32),
                pltpu.VMEM((NT, 2 * T, 128), F32),
                pltpu.VMEM((4, W4, 3 * D), BF16),
                pltpu.VMEM((4, W4, D), BF16),
                pltpu.VMEM((7, 4, W2 // 2, 128), U32),
                pltpu.VMEM((3, 7, 4, W2 // 2, 128), U32),
                pltpu.VMEM((4, 49, 2, W4 // 2, 128), U32),
                pltpu.VMEM((NT, S, 128), F32),
                pltpu.VMEM((NT, CH, 128), F32),
                pltpu.VMEM((NT, HALO + CH, 128), F32),
                pltpu.VMEM((NT, HALO + CH, 128), F32),
                pltpu.VMEM((NT, S // 2, 128), U32),
                pltpu.VMEM((S // 128, D // 2, 128), U32),
                pltpu.VMEM((S // 128, D // 2, 128), U32),
                pltpu.VMEM((NU, 8, QB), F32),
                pltpu.VMEM((NU, DH, QB), F32),
                pltpu.VMEM((NB, D // DH * 8, 128), F32),
                pltpu.VMEM((D // DH, 256), F32),
                pltpu.VMEM((NU, QT, DH, 256), F32),
                pltpu.VMEM((256, 128), F32),
                pltpu.SemaphoreType.DMA((NB,)),
                pltpu.SemaphoreType.DMA((NP + NQ + S // CH + 1,)),
                pltpu.SemaphoreType.DMA((NQB,)),
            ],
            compiler_params=pltpu.CompilerParams(vmem_limit_bytes=127 * 2 ** 20, flags=flags),
            name=name,
        )(A_x.reshape(S, D), A_wqkv.reshape(2, W2, 3 * D), A_wo.reshape(8, 2, 2 * DH, D),
          B_wqkv.reshape(4, W4, 3 * D), B_wo.reshape(4, W4, D))
        return out.reshape(1, S, D)

    fn.__name__ = name
    return jax.jit(fn)


pallas_interleave_layers__sliding_local_dilated__softmax_full_mha__prompt_kernel = make(
    name="pallas_interleave_layers__sliding_local_dilated__softmax_full_mha__prompt_kernel", )
```

```python
import functools
import math

import jax
import jax.numpy as jnp
from jax import lax
import jax.experimental.pallas as pl
import jax.experimental.pallas.tpu as pltpu

S = 2048
D = 1024
DH = 32
WIN, DIL = 8, 2
HALO = 16
NT = D // 128
W2, W4 = D // 2, D // 4
HT = 64
T = 2 * HT
NB = S // T
CH = 2 * T
NCH = S // CH
QS = 4
NQ = 4
AHEAD = 2
QB = 512
QT = QB // 128
NQB = S // QB
KC = 128
NU = 128 // DH
QSCALE = (DH ** -0.5) * math.log2(math.e)
MASKED = -1e9 * math.log2(math.e)
F32, BF16, U32 = jnp.float32, jnp.bfloat16, jnp.uint32
WQ, WK, WV, WO = range(4)

LHS = (((1, 0, 0), (1, 1, 1)), ((1, 1, 0), (1, 1, 1)), ((1, 0, 0),), ((1, 1, 1),),
       ((1, 0, 0), (1, 0, 1)), ((1, 1, 0), (-1, 0, 0)), ((1, 0, 1), (-1, 1, 1)))
RHS = (((1, 0, 0), (1, 1, 1)), ((1, 0, 0),), ((1, 0, 1), (-1, 1, 1)), ((1, 1, 0), (-1, 0, 0)),
       ((1, 1, 1),), ((1, 0, 0), (1, 0, 1)), ((1, 1, 0), (1, 1, 1)))
ORDER = (0, 3, 4, 6, 2, 1, 5)


def _combine(m):
    return ((m[0] + m[3] - m[4] + m[6], m[4] + m[2]), (m[3] + m[1], m[0] + m[2] - m[1] + m[5]))


def _signed_sum(terms, block):
    total = block(*terms[0][1:])
    for sign, i, j in terms[1:]:
        total = total + block(i, j) if sign > 0 else total - block(i, j)
    return total


def _operands(table, block):
    grid = {(i, j): block(i, j) for i in range(2) for j in range(2)}
    return _pack(jnp.stack([_signed_sum(terms, lambda i, j: grid[i, j]) for terms in table]).astype(BF16))


def _operands2(table, block, r):
    return _operands(table, lambda i, j: _signed_sum(table[r], lambda a, b: block(2 * a + i, 2 * b + j)))


def _pack(x):
    return pltpu.bitcast(x, U32)


def _unpack(x):
    return pltpu.bitcast(x, BF16)


def _now(x):
    return x


def _rows(i, n):
    return pl.ds(i * n if isinstance(i, int) else pl.multiple_of(i * n, n), n)


def _bit_clear(shape, axis, bit):
    return (lax.broadcasted_iota(jnp.int32, shape, axis) & bit) == 0


def _swap_lane_bits(tiles):
    last = tiles[0].ndim - 1
    t = [tiles[j] if j == 0 else pltpu.roll(tiles[j], 4 * j, last) for j in range(8)]
    t = [t[-f % 8] for f in range(8)]
    for b in range(3):
        clear = _bit_clear(t[0].shape, last, 4 << b)
        t = [lax.select(clear, t[f], t[(f - (1 << b)) % 8]) for f in range(8)]
    return [t[f] if f == 0 else pltpu.roll(t[f], 128 - 4 * f, last) for f in range(8)]


def _swap_sublane_bits(v):
    for bit, s in ((2, 4), (1, 2)):
        clear = _bit_clear((8, 128), 0, s)
        new = list(v)
        for r in range(4):
            if not r & bit:
                new[r] = lax.select(clear, v[r], pltpu.roll(v[r | bit], s, 0))
                new[r | bit] = lax.select(clear, pltpu.roll(v[r], 8 - s, 0), v[r | bit])
        v = new
    return v


class _Pacer:
    def __init__(self, index):
        self.never = index < 0
        self.masks = {}
        self.slot = 0
        self.todo = []

    def add(self, tasks, span, delay=0):
        for k, task in enumerate(tasks):
            self.todo.append((self.slot + delay + k * span // len(tasks), task))

    def _run(self, after):
        due = [t for s, t in self.todo if s < self.slot]
        self.todo = [(s, t) for s, t in self.todo if s >= self.slot]
        for task in due:
            task(after)

    def overdue(self):
        self._run(_now)

    def tick(self, result, row=0):
        seen = {}

        def after(x):
            if x.shape not in self.masks:
                self.masks[x.shape] = jnp.broadcast_to(self.never, x.shape)
            if (x.shape, x.dtype) not in seen:
                r = result[row:row + x.shape[-2], :128]
                r = r if x.dtype == F32 else pltpu.bitcast(r, x.dtype)
                seen[x.shape, x.dtype] = jnp.broadcast_to(r, x.shape)
            return lax.select(self.masks[x.shape], seen[x.shape, x.dtype], x)
        self.slot += 1
        self._run(after)


def _kernel(x_hbm, wa_hbm, woa_hbm, wb_hbm, wob_hbm, out_hbm,
            xio, xres, xop, top, bop, xn, raw_b, raw_ob, wq, wa, wb,
            qa, pa, ka, va, kb, qtb, vtb, mbuf, abuf, lbuf, linv, qf, kf, sems):

    def weight_a(mat, half):
        return wq.at[half] if mat == WQ else wa.at[mat - WK, half]

    def matmul_a(src, mat, emit, pacer):
        for n in range(NT // 2):
            m = {}
            for r in ORDER:
                m[r] = jnp.dot(_unpack(src[r]), _unpack(weight_a(mat, n >> 1)[r, :, _rows(n & 1, 128)]),
                               preferred_element_type=F32)
                pacer.tick(m[r])
            c = _combine(m)
            for j in range(2):
                emit(n + j * (NT // 2), jnp.concatenate([c[0][j], c[1][j]], axis=0))

    def products_b(src, mat, emit, pacer):
        for n in range(NT // 4):
            outer = {}
            for r1 in ORDER:
                m = {}
                for r2 in ORDER:
                    m[r2] = jnp.dot(_unpack(src[7 * r1 + r2]), _unpack(wb[mat, 7 * r1 + r2, :, _rows(n, 128)]),
                                    preferred_element_type=F32)
                    pacer.tick(m[r2])
                    yield
                outer[r1] = _combine(m)
            c = [[_combine({r: outer[r][i][j] for r in ORDER}) for j in range(2)] for i in range(2)]
            for j in range(4):
                emit(n + j * (NT // 4),
                     jnp.concatenate([c[i % 2][j % 2][i // 2][j // 2] for i in range(4)], axis=0))

    def stage_tasks(dsts, g, src, make_rows):
        def block(r, t, after):
            return lambda i, j: after(src[t + j * (NT // g), pl.ds(i * HT + r, 16), :])

        def store(k, r, t, ops):
            for dst in dsts:
                dst[pl.ds(k, 7), _rows(r // 16, 8), _rows(t, 128)] = ops

        def stage(r, after):
            for t in range(NT // g):
                store(0, r, t, _operands(LHS, block(r, t, after)))

        def stage2(r, t, r1, after):
            store(7 * r1, r, t, _operands2(LHS, block(r, t, after), r1))

        if make_rows is None:
            return [functools.partial(stage2, r, t, r1)
                    for r1 in ORDER for t in range(NT // g) for r in range(0, HT, 16)]
        tasks = []
        for r in range(0, HT + 16, 16):
            if r < HT:
                tasks += [functools.partial(make_rows, i * HT + r + dr) for i in range(g) for dr in (0, 8)]
            if r > 0 and g == 2:
                tasks.append(functools.partial(stage, r - 16))
            elif r > 0:
                tasks += [functools.partial(stage2, r - 16, t, r1) for t in range(NT // g) for r1 in ORDER]
        return tasks

    def norm_tasks(dsts, g, i, slot=0, fresh=False):
        x = xres.at[:, _rows(i, g * HT)]
        y = xn.at[:, _rows(slot, g * HT)]
        mean = {}

        def means(r0, after):
            for r in (r0, r0 + HT):
                if fresh:
                    v = xio.at[_rows(i, g * HT)][pl.ds(r, 16), :].astype(F32)
                    x[:, pl.ds(r, 16), :] = jnp.stack([v[:, t * 128:(t + 1) * 128] for t in range(NT)])
                for rr in (r, r + 8):
                    total = after(jnp.sum(x[:, pl.ds(rr, 8), :], axis=0))
                    mean[rr] = jnp.sum(total, axis=-1, keepdims=True) * (1.0 / D)

        def norm(r, after):
            c = x[:, pl.ds(r, 8), :] - after(jnp.broadcast_to(mean[r], (8, 128)))[None]
            var = jnp.sum(jnp.sum(c * c, axis=0), axis=-1, keepdims=True) * (1.0 / D)
            y[:, pl.ds(r, 8), :] = c * lax.rsqrt(var + 1e-5)[None]
        return ([functools.partial(means, k + r) for r in range(0, HT, 16) for k in range(0, g * HT, T)]
                + stage_tasks(dsts, g, y, norm))

    def prep_a(mat, raw, i, n, after):
        w = _swap_lane_bits([after(_pack(raw[:, _rows(i, n), _rows(mat * NT + j, 128)])) for j in range(NT)])
        for t in range(NT // 2):
            weight_a(mat, t >> 1)[:, _rows(i, n // 2), _rows(t & 1, 128)] = _operands(
                RHS, lambda k, j: _unpack(w[t + j * (NT // 2)][k]).astype(F32))

    def prep_b_tasks(mat, i):
        raw, tile0 = (raw_ob, 0) if mat == WO else (raw_b, mat * NT)
        src, dst = _rows(i, 16), _rows(i, 8)

        def task(t, r1, after):
            def block(k, j):
                return _unpack(after(_pack(raw[k, src, _rows(tile0 + t + j * (NT // 4), 128)]))).astype(F32)
            wb.at[mat][pl.ds(7 * r1, 7), dst, _rows(t, 128)] = _operands2(RHS, block, r1)
        return [functools.partial(task, t, r1) for t in range(NT // 4) for r1 in ORDER]

    def first_norm(fresh):
        for task in norm_tasks((top.at[0], xop.at[0]), 2, 0, 0, fresh):
            task(_now)

    def query_body(c, n, pacer, fresh):
        for j in range(n):
            nxt = c * n + j + 1
            if j == n - 1:
                nxt = jnp.minimum(nxt, NB - 1)
            pacer.add(norm_tasks((top.at[(j + 1) % n], xop.at[nxt]), 2, nxt, j % 2, fresh), 22)
            r = _rows(c * n + j, T)

            def emit(t, y):
                qa[t, r, :] = y * QSCALE
            matmul_a(top.at[j], WQ, emit, pacer)
        assert not pacer.todo

    def window_body(c):
        pacer = _Pacer(c)
        q_chunk = qa.at[:, _rows(c, CH)]
        x_chunk = xres.at[:, _rows(c, CH)]
        clear = {s: _bit_clear((WIN, 8, 128), 2, s) for s in (1, 2)}

        def project(mat, dst, j):
            def emit(t, y):
                dst[t, pl.ds(HALO + j * T, T), :] = y
                if j == 0:
                    first = jnp.broadcast_to(y[0:1], (HALO, 128))
                    dst[t, pl.ds(0, HALO), :] = jnp.where(c == 0, first, dst[t, pl.ds(CH, HALO), :])
            matmul_a(xop.at[2 * c + j], mat, emit, pacer)

        def pair_sum(x, s):
            return x + lax.select(clear[s], pltpu.roll(x, 128 - s, 2), pltpu.roll(x, s, 2))

        def logits(r, after):
            q = after(q_chunk[:, pl.ds(r, 8), :])
            x = jnp.stack([jnp.sum(q * ka[:, pl.ds(HALO + r - DIL * w, 8), :], axis=0) for w in range(WIN)])
            pa[:, pl.ds(r, 8), :] = pair_sum(x, 2)

        def softmax(r, after):
            x = pair_sum(after(pa[:, pl.ds(r, 8), :]), 1)
            if r < DIL * (WIN - 1):
                pos = c * CH + r + lax.broadcasted_iota(jnp.int32, x.shape, 1)
                x = jnp.where(pos >= DIL * lax.broadcasted_iota(jnp.int32, x.shape, 0), x, MASKED)
            e = jnp.exp2(x - jnp.max(x, axis=0, keepdims=True))
            pa[:, pl.ds(r, 8), :] = e * (1.0 / jnp.sum(e, axis=0, keepdims=True))

        def mix(j, r, after):
            r += j * T
            e = after(pa[:, pl.ds(r, 8), :])
            pa[:, pl.ds(r, 8), :] = functools.reduce(
                jnp.add, [e[w:w + 1] * va[:, pl.ds(HALO + r - DIL * w, 8), :] for w in range(WIN)])

        def project_out(j):
            def emit(t, y):
                x_chunk[t, _rows(j, T), :] = x_chunk[t, _rows(j, T), :] + y
            matmul_a(top.at[j], WO, emit, pacer)

        order = [r + dr for r in range(0, HT, 16) for dr in (0, 8, HT, HT + 8)]
        for j in range(2):
            pacer.add([functools.partial(logits, j * T + r) for r in order], 16, 28 * (j + 1))
            pacer.add([functools.partial(softmax, j * T + r) for r in order], 12, 28 * (j + 1) + 16)
            pacer.add(stage_tasks((top.at[j],), 2, pa.at[:, _rows(j, T)], functools.partial(mix, j)),
                      26, 28 * (j + 3))
            pacer.add([t for m in (WQ, WK, WV) for t in prep_b_tasks(m, 2 * c + j)], 26 - 2 * j, 140 * j)
        for mat, dst in ((WK, ka), (WV, va)):
            for j in range(2):
                project(mat, dst, j)
        for j in range(2):
            project_out(j)
        assert not pacer.todo

    def qkv_body(c):
        pacer = _Pacer(c)
        for j in range(2):
            i = 2 * c + j
            pacer.add(norm_tasks((bop.at[1 - j],), 4, jnp.minimum(i + 1, NCH - 1)), 250)
            for mat in (WQ, WV, WK):
                def emit(g, y):
                    if mat == WK:
                        kb[g, _rows(i, CH // 2), :] = _pack(y.astype(BF16))
                        return
                    y = (y * QSCALE if mat == WQ else y).astype(BF16)
                    for k in range(2):
                        (qtb if mat == WQ else vtb)[2 * i + k, _rows(g, 64), :] = _pack(y[k * T:(k + 1) * T].T)
                for _ in products_b(bop.at[j], mat, emit, pacer):
                    pass
        assert not pacer.todo

    def out_t(qb, a, head, n=1):
        return qa.at[qb * (QT // 2) + a // 2, _rows((a % 2) * (D // DH // n) + head, n * DH)]

    def attend(sbuf, i, pacer, nv, do_pv, do_scores, between=None):
        on_vpu = [k * (S // KC) // nv for k in range(nv)]
        m_next = [None] * NU
        part = {}

        def keep(u, r, s):
            sbuf[u, pl.ds(r, s.shape[0]), :] = s
            m = jnp.max(s.reshape(-1, 8, QB), axis=0)
            m_next[u] = m if m_next[u] is None else jnp.maximum(m_next[u], m)

        def vpu_scores(u, r, d0, after):
            k = after(kf[_rows(r, 8), :])
            for d in range(d0, d0 + 4):
                kd = jnp.broadcast_to(k[:, u * DH + d:u * DH + d + 1], (QT, 8, 128))
                term = kd * jnp.broadcast_to(qf[u, :, pl.ds(d, 1), pl.ds(0, 128)], (QT, 8, 128))
                part[u] = term if d == 0 else part[u] + term
            if d0 + 4 == DH:
                keep(u, on_vpu[r // 2] * KC + (r % 2) * 8,
                     jnp.concatenate([part[u][a] for a in range(QT)], axis=1))

        if do_scores:
            gn, qbn = (i + 1) & (NT - 1), (i + 1) >> 3
            qm = []
            for u in range(NU):
                qh = _unpack(qtb[_rows(qbn, QT), _rows(gn * NU + u, DH // 2), :])
                qf[u, :, :, pl.ds(0, 128)] = qh.astype(F32)
                heads = [jnp.zeros((DH, QB), BF16)] * NU
                heads[u] = jnp.concatenate([qh[a] for a in range(QT)], axis=1)
                qm.append(jnp.concatenate(heads, axis=0))
            for j, c in enumerate(on_vpu):
                kf[_rows(j, 16), :] = _unpack(kb[gn, _rows(c * (KC // 16), 8), :]).astype(F32)
            pacer.add([functools.partial(vpu_scores, u, r, d0)
                       for u in range(NU) for r in range(2 * nv) for d0 in range(0, DH, 4)],
                      NU * (S - 16 * nv) // 8, -12)
        for u in range(NU):
            if do_pv:
                head = (i & (NT - 1)) * NU + u
                v_rows = _rows(head, DH // 2)
                m = jnp.broadcast_to(jnp.max(mbuf[u], axis=0, keepdims=True), (8, QB))[None]
                l = None
            for c in range(S // KC):
                if do_pv:
                    sc = sbuf[u, _rows(c, KC), :].reshape(KC // 8, 8, QB)
                if do_scores:
                    pacer.overdue()
                    skip = 16 if c in on_vpu else 0
                    keys = _unpack(kb[gn, pl.ds((c * KC + skip) // 2, (KC - skip) // 2), :])
                    s = jnp.dot(keys, qm[u], preferred_element_type=F32)
                    keep(u, c * KC + skip, s)
                    for r in range(0, KC - skip, 8):
                        pacer.tick(s, r)
                if do_pv:
                    p = jnp.exp2(sc - m).reshape(KC, QB)
                    for r in reversed(range(0, KC, 8)):
                        l = p[r:r + 8] if l is None else l + p[r:r + 8]
                    pv = jnp.dot(_unpack(vtb[c, v_rows, :]), p.astype(BF16), preferred_element_type=F32)
                    acc = pv if c == 0 else abuf[u] + pv
                    if c + 1 < S // KC:
                        abuf[u] = acc
                if between is not None:
                    between()
            if do_pv:
                for a in range(QT):
                    lbuf[(i >> 3) * QT + a, _rows(head, 8), :] = l[:, a * 128:(a + 1) * 128]
                    out_t(i >> 3, a, head)[...] = acc[:, a * 128:(a + 1) * 128]
        if do_scores:
            assert not pacer.todo
            for u in range(NU):
                mbuf[u] = m_next[u]

    def out_stage_tasks(qb, j):
        def invert(a, after):
            l = [lbuf[qb * QT + 2 * j + a, pl.ds(k, D // DH, stride=8), :] for k in range(8)]
            linv[:, _rows(a, 128)] = 1.0 / after(functools.reduce(jnp.add, l))

        def normalise(a, g, after):
            inv = after(jnp.stack([jnp.broadcast_to(linv[pl.ds(NU * g + u, 1), _rows(a, 128)], (8, 128))
                                   for u in range(NU)]))
            o = out_t(qb, 2 * j + a, g, NU)[...].reshape(NU, DH // 8, 8, 128) * inv[:, None]
            xn[g, _rows(a, T), :] = o.reshape(128, 128).T
        return ([functools.partial(invert, a) for a in range(2)]
                + [functools.partial(normalise, a, g) for t in range(2) for g in range(t, NT, 2) for a in range(2)],
                stage_tasks((bop.at[j],), 4, xn, None))

    def out_products(qb, nxt, pacer):
        for j in range(2):
            first, second = out_stage_tasks(nxt, 0) if j else out_stage_tasks(qb, 1)
            pacer.add(first, 22)
            pacer.add(second, 74, 22)
            r = _rows(2 * qb + j, CH)

            def emit(t, y):
                x = xres[t, r, :] + y
                xres[t, r, :] = x
                xio[r, _rows(t, 128)] = x.astype(BF16)
            yield from products_b(bop.at[j], WO, emit, pacer)
        assert not pacer.todo

    def attention(rep, sbuf):
        steps = NQB * NT
        pacer = _Pacer(rep)
        pacer.add([t for i in range(W4 // 16) for t in prep_b_tasks(WO, i)], 230 * NU)
        attend(sbuf, -1, pacer, 4, False, True)
        pl.loop(0, steps - 1)(lambda i: attend(sbuf, i, _Pacer(i), 6, True, True))

        for tasks in out_stage_tasks(0, 0):
            for task in tasks:
                task(_now)
        out = out_products(0, 1, _Pacer(rep))
        count = [-12, 0]

        def between():
            count[0] += 1
            while count[1] * (NU * (S // KC) - 12) < count[0] * 190:
                next(out)
                count[1] += 1
        attend(sbuf, steps - 1, None, 0, True, False, between)
        for _ in out:
            pass

    def copy(src, dst, idx, sem):
        return pltpu.make_async_copy(src.at[idx], dst.at[idx], sems.at[sem])

    def b_copy(c):
        return copy(wb_hbm, raw_b, (slice(None), _rows(c, W4 // NCH)), NCH + NQ + c)

    def bo_copy():
        return copy(wob_hbm, raw_ob, (slice(None),), 2 * NCH + NQ)

    def out_copy(c):
        return copy(xio, out_hbm, (_rows(c, QB),), c)

    def start_up(raw_a, raw_oa):
        step_rows = W2 // NCH

        def q_copy(i):
            return copy(wa_hbm, raw_a, (slice(None), _rows(i, W2 // NQ), pl.ds(0, D)), NCH + i)

        def o_tiles(i):
            return (i & 3, (i & 3) + 4)

        def step_copies(i, last):
            x_rows = pl.ds(_rows(2 * i + 1, T).start, T if last else 2 * T)
            return [copy(x_hbm, xio, (x_rows,), i),
                    copy(wa_hbm, raw_a, (slice(None), _rows(i, step_rows), pl.ds(D, 2 * D)), i)] + [
                copy(woa_hbm, raw_oa, (slice(None), i >> 2, slice(None), _rows(j, 128)), i) for j in o_tiles(i)]

        def start_step(i, last=False):
            for c in step_copies(i, last):
                c.start()
            if last:
                b_copy(0).start()

        def wait_step(i, last=False):
            for c in step_copies(i, last):
                c.wait()

        def prep_o(i, h4, h0, after):
            b = [[_swap_sublane_bits(
                [after(_pack(raw_oa[h4 * 4 + h, i >> 2, _rows(2 * h0 + d4, 16), _rows(j, 128)])) for h in range(4)])
                for j in o_tiles(i)] for d4 in range(2)]
            for d in range(4):
                rows = _rows(d * 8 + (i >> 2) * 4 + h0 * 2 + h4, 8)
                weight_a(WO, (i & 3) >> 1)[:, rows, _rows(i & 1, 128)] = _operands(
                    RHS, lambda k, j: _unpack(b[k][j][d]).astype(F32))

        x_first = copy(x_hbm, xio, (_rows(0, T),), NCH - 1)
        x_first.start()
        for i in range(NQ):
            q_copy(i).start()
        for i in range(AHEAD):
            start_step(i)
        for buf in (ka, va):
            buf[:, pl.ds(CH, HALO), :] = jnp.zeros((NT, HALO, 128), F32)
        x_first.wait()
        first_norm(True)

        @pl.loop(0, NQ)
        def _(i):
            q_copy(i).wait()
            prep_a(WQ, raw_a, i, W2 // NQ, _now)

        @pl.loop(0, NCH)
        def _(i):
            pl.when(i + AHEAD < NCH - 1)(lambda: start_step(i + AHEAD))
            pl.when(i + AHEAD == NCH - 1)(lambda: start_step(NCH - 1, True))
            pl.when(i < NCH - 1)(lambda: wait_step(i))
            pl.when(i == NCH - 1)(lambda: wait_step(NCH - 1, True))
            pacer = _Pacer(i)
            pacer.add([functools.partial(prep_a, m, raw_a, i * (step_rows // 16) + k, 16)
                       for k in range(step_rows // 16) for m in (WK, WV)], 30, 20)
            pacer.add([functools.partial(prep_o, i, k // 2, k % 2) for k in range(4)], 20, -1)
            pacer.overdue()
            query_body(i, 2, pacer, True)

    pl.run_scoped(start_up, pltpu.VMEM((2, W2, 3 * D), BF16), pltpu.VMEM((8, 2, 2 * DH, D), BF16))
    for c in range(1, NCH):
        b_copy(c).start()
    bo_copy().start()

    @pl.loop(0, 2)
    def _(rep):
        @pl.loop(0, NCH)
        def _(c):
            pl.when(rep == 0)(lambda: b_copy(c).wait())
            window_body(c)

        pl.when(rep == 0)(lambda: bo_copy().wait())
        for task in norm_tasks((bop.at[0],), 4, 0):
            task(_now)
        pl.loop(0, NCH // 2)(qkv_body)
        pl.run_scoped(functools.partial(attention, rep), pltpu.VMEM((NU, S, QB), F32))
        pl.when(rep == 1)(lambda: out_copy(0).start())

        @pl.loop(1, NQB)
        def _(c):
            for _ in out_products(c, jnp.minimum(c + 1, NQB - 1), _Pacer(c)):
                pass
            pl.when(rep == 1)(lambda: out_copy(c).start())

        @pl.when(rep == 0)
        def _():
            first_norm(False)
            pl.loop(0, NB // QS)(lambda c: query_body(c, QS, _Pacer(c), False))

    for c in range(NQB):
        out_copy(c).wait()


@jax.jit
def pallas_interleave_layers__sliding_local_dilated__softmax_full_mha__prompt_kernel(
    A_x: jax.Array,
    A_wqkv: jax.Array,
    A_wo: jax.Array,
    B_x: jax.Array,
    B_wqkv: jax.Array,
    B_wo: jax.Array,
):
    del B_x
    hbm = pl.BlockSpec(memory_space=pltpu.HBM)
    out = pl.pallas_call(
        _kernel,
        out_shape=jax.ShapeDtypeStruct((S, D), BF16),
        in_specs=[hbm] * 5,
        out_specs=hbm,
        scratch_shapes=[
            pltpu.VMEM((S, D), BF16),
            pltpu.VMEM((NT, S + 8, 128), F32),
            pltpu.VMEM((NB, 7, HT // 2, W2), U32),
            pltpu.VMEM((QS, 7, HT // 2, W2), U32),
            pltpu.VMEM((2, 49, HT // 2, W4), U32),
            pltpu.VMEM((NT, CH + 8, 128), F32),
            pltpu.VMEM((4, W4, 3 * D), BF16),
            pltpu.VMEM((4, W4, D), BF16),
            pltpu.VMEM((2, 7, W2 // 2, 256), U32),
            pltpu.VMEM((3, 2, 7, W2 // 2, 256), U32),
            pltpu.VMEM((4, 49, W4 // 2, W4), U32),
            pltpu.VMEM((NT, S + 8, 128), F32),
            pltpu.VMEM((NT, CH + 8, 128), F32),
            pltpu.VMEM((NT, HALO + CH + 8, 128), F32),
            pltpu.VMEM((NT, HALO + CH + 8, 128), F32),
            pltpu.VMEM((NT, S // 2, 128), U32),
            pltpu.VMEM((S // 128, D // 2, 128), U32),
            pltpu.VMEM((S // 128, D // 2, 128), U32),
            pltpu.VMEM((NU, 8, QB), F32),
            pltpu.VMEM((NU, DH, QB), F32),
            pltpu.VMEM((NB, D // DH * 8 + 8, 128), F32),
            pltpu.VMEM((D // DH, 256), F32),
            pltpu.VMEM((NU, QT, DH, 256), F32),
            pltpu.VMEM((128, 128), F32),
            pltpu.SemaphoreType.DMA((2 * NCH + NQ + 1,)),
        ],
        compiler_params=pltpu.CompilerParams(vmem_limit_bytes=127 * 2 ** 20),
        name="interleave_layers",
    )(A_x.reshape(S, D), A_wqkv.reshape(2, W2, 3 * D), A_wo.reshape(8, 2, 2 * DH, D),
      B_wqkv.reshape(4, W4, 3 * D), B_wo.reshape(4, W4, D))
    return out.reshape(1, S, D)
```

```python
import functools
import math

import jax
import jax.numpy as jnp
from jax import lax
import jax.experimental.pallas as pl
import jax.experimental.pallas.tpu as pltpu

S = 2048
D = 1024
DH = 32
WIN, DIL = 8, 2
HALO = 16
NT = D // 128
W2, W4 = D // 2, D // 4
HT = 64
T = 2 * HT
NB = S // T
CH = 2 * T
NCH = S // CH
QS = 4
NQ = 4
AHEAD = 2
QB = 512
QT = QB // 128
NQB = S // QB
KC = 128
NU = 128 // DH
NV = 6
QSCALE = (DH ** -0.5) * math.log2(math.e)
MASKED = -1e9 * math.log2(math.e)
F32, BF16, U32 = jnp.float32, jnp.bfloat16, jnp.uint32
WQ, WK, WV, WO = range(4)

LHS = (((1, 0, 0), (1, 1, 1)), ((1, 1, 0), (1, 1, 1)), ((1, 0, 0),), ((1, 1, 1),),
       ((1, 0, 0), (1, 0, 1)), ((1, 1, 0), (-1, 0, 0)), ((1, 0, 1), (-1, 1, 1)))
RHS = (((1, 0, 0), (1, 1, 1)), ((1, 0, 0),), ((1, 0, 1), (-1, 1, 1)), ((1, 1, 0), (-1, 0, 0)),
       ((1, 1, 1),), ((1, 0, 0), (1, 0, 1)), ((1, 1, 0), (1, 1, 1)))
ORDER = (0, 3, 4, 6, 2, 1, 5)


def _combine(m):
    return ((m[0] + m[3] - m[4] + m[6], m[4] + m[2]), (m[3] + m[1], m[0] + m[2] - m[1] + m[5]))


def _signed_sum(terms, block):
    total = block(*terms[0][1:])
    for sign, i, j in terms[1:]:
        total = total + block(i, j) if sign > 0 else total - block(i, j)
    return total


def _operands(table, block):
    grid = {(i, j): block(i, j) for i in range(2) for j in range(2)}
    return _pack(jnp.stack([_signed_sum(terms, lambda i, j: grid[i, j]) for terms in table]).astype(BF16))


def _operands2(table, block, r):
    return _operands(table, lambda i, j: _signed_sum(table[r], lambda a, b: block(2 * a + i, 2 * b + j)))


def _pack(x):
    return pltpu.bitcast(x, U32)


def _unpack(x):
    return pltpu.bitcast(x, BF16)


def _now(x):
    return x


def _rows(i, n):
    return pl.ds(i * n if isinstance(i, int) else pl.multiple_of(i * n, n), n)


def _bit_clear(shape, axis, bit):
    return (lax.broadcasted_iota(jnp.int32, shape, axis) & bit) == 0


def _swap_lane_bits(tiles):
    last = tiles[0].ndim - 1
    t = [tiles[j] if j == 0 else pltpu.roll(tiles[j], 4 * j, last) for j in range(8)]
    t = [t[-f % 8] for f in range(8)]
    for b in range(3):
        clear = _bit_clear(t[0].shape, last, 4 << b)
        t = [lax.select(clear, t[f], t[(f - (1 << b)) % 8]) for f in range(8)]
    return [t[f] if f == 0 else pltpu.roll(t[f], 128 - 4 * f, last) for f in range(8)]


def _swap_sublane_bits(v):
    for bit, s in ((2, 4), (1, 2)):
        clear = _bit_clear((8, 128), 0, s)
        new = list(v)
        for r in range(4):
            if not r & bit:
                new[r] = lax.select(clear, v[r], pltpu.roll(v[r | bit], s, 0))
                new[r | bit] = lax.select(clear, pltpu.roll(v[r], 8 - s, 0), v[r | bit])
        v = new
    return v


class _Pacer:
    def __init__(self, index):
        self.never = index < 0
        self.masks = {}
        self.slot = 0
        self.todo = []

    def add(self, tasks, span, delay=0):
        for k, task in enumerate(tasks):
            self.todo.append((self.slot + delay + k * span // len(tasks), task))

    def _run(self, after):
        due = [t for s, t in self.todo if s < self.slot]
        self.todo = [(s, t) for s, t in self.todo if s >= self.slot]
        for task in due:
            task(after)

    def overdue(self):
        self._run(_now)

    def tick(self, result, row=0):
        seen = {}

        def after(x):
            if x.shape not in self.masks:
                self.masks[x.shape] = jnp.broadcast_to(self.never, x.shape)
            if (x.shape, x.dtype) not in seen:
                r = result[row:row + x.shape[-2], :128]
                r = r if x.dtype == F32 else pltpu.bitcast(r, x.dtype)
                seen[x.shape, x.dtype] = jnp.broadcast_to(r, x.shape)
            return lax.select(self.masks[x.shape], seen[x.shape, x.dtype], x)
        self.slot += 1
        self._run(after)


def _kernel(x_hbm, wa_hbm, woa_hbm, wb_hbm, wob_hbm, out_hbm,
            xio, xres, xop, top, bop, xn, raw_b, raw_ob, wq, wa, wb,
            qa, pa, ka, va, kb, qtb, vtb, mbuf, abuf, lbuf, linv, qf, kf, sems):

    def weight_a(mat, half):
        return wq.at[half] if mat == WQ else wa.at[mat - WK, half]

    def matmul_a(src, mat, emit, pacer):
        for n in range(NT // 2):
            m = {}
            for r in ORDER:
                m[r] = jnp.dot(_unpack(src[r]), _unpack(weight_a(mat, n >> 1)[r, :, _rows(n & 1, 128)]),
                               preferred_element_type=F32)
                pacer.tick(m[r])
            c = _combine(m)
            for j in range(2):
                emit(n + j * (NT // 2), jnp.concatenate([c[0][j], c[1][j]], axis=0))

    def products_b(src, mat, emit, pacer):
        for n in range(NT // 4):
            outer = {}
            for r1 in ORDER:
                m = {}
                for r2 in ORDER:
                    m[r2] = jnp.dot(_unpack(src[7 * r1 + r2]), _unpack(wb[mat, 7 * r1 + r2, :, _rows(n, 128)]),
                                    preferred_element_type=F32)
                    pacer.tick(m[r2])
                    yield
                outer[r1] = _combine(m)
            c = [[_combine({r: outer[r][i][j] for r in ORDER}) for j in range(2)] for i in range(2)]
            for j in range(4):
                emit(n + j * (NT // 4),
                     jnp.concatenate([c[i % 2][j % 2][i // 2][j // 2] for i in range(4)], axis=0))

    def stage_tasks(dsts, g, src, make_rows):
        def block(r, t, after):
            return lambda i, j: after(src[t + j * (NT // g), pl.ds(i * HT + r, 16), :])

        def store(k, r, t, ops):
            for dst in dsts:
                dst[pl.ds(k, 7), _rows(r // 16, 8), _rows(t, 128)] = ops

        def stage(r, after):
            for t in range(NT // g):
                store(0, r, t, _operands(LHS, block(r, t, after)))

        def stage2(r, t, r1, after):
            store(7 * r1, r, t, _operands2(LHS, block(r, t, after), r1))

        if make_rows is None:
            return [functools.partial(stage2, r, t, r1)
                    for r1 in ORDER for t in range(NT // g) for r in range(0, HT, 16)]
        tasks = []
        for r in range(0, HT + 16, 16):
            if r < HT:
                tasks += [functools.partial(make_rows, i * HT + r + dr) for i in range(g) for dr in (0, 8)]
            if r > 0 and g == 2:
                tasks.append(functools.partial(stage, r - 16))
            elif r > 0:
                tasks += [functools.partial(stage2, r - 16, t, r1) for t in range(NT // g) for r1 in ORDER]
        return tasks

    def norm_tasks(dsts, g, i, slot=0, fresh=False):
        x = xres.at[:, _rows(i, g * HT)]
        y = xn.at[:, _rows(slot, g * HT)]
        mean = {}

        def means(r0, after):
            for r in (r0, r0 + HT):
                if fresh:
                    v = xio.at[_rows(i, g * HT)][pl.ds(r, 16), :].astype(F32)
                    x[:, pl.ds(r, 16), :] = jnp.stack([v[:, t * 128:(t + 1) * 128] for t in range(NT)])
                for rr in (r, r + 8):
                    total = after(jnp.sum(x[:, pl.ds(rr, 8), :], axis=0))
                    mean[rr] = jnp.sum(total, axis=-1, keepdims=True) * (1.0 / D)

        def norm(r, after):
            c = x[:, pl.ds(r, 8), :] - after(jnp.broadcast_to(mean[r], (8, 128)))[None]
            var = jnp.sum(jnp.sum(c * c, axis=0), axis=-1, keepdims=True) * (1.0 / D)
            y[:, pl.ds(r, 8), :] = c * lax.rsqrt(var + 1e-5)[None]
        return ([functools.partial(means, k + r) for r in range(0, HT, 16) for k in range(0, g * HT, T)]
                + stage_tasks(dsts, g, y, norm))

    def prep_a(mat, raw, i, n, after):
        w = _swap_lane_bits([after(_pack(raw[:, _rows(i, n), _rows(mat * NT + j, 128)])) for j in range(NT)])
        for t in range(NT // 2):
            weight_a(mat, t >> 1)[:, _rows(i, n // 2), _rows(t & 1, 128)] = _operands(
                RHS, lambda k, j: _unpack(w[t + j * (NT // 2)][k]).astype(F32))

    def prep_b_tasks(mat, i):
        raw, tile0 = (raw_ob, 0) if mat == WO else (raw_b, mat * NT)
        src, dst = _rows(i, 16), _rows(i, 8)

        def task(t, r1, after):
            def block(k, j):
                return _unpack(after(_pack(raw[k, src, _rows(tile0 + t + j * (NT // 4), 128)]))).astype(F32)
            wb.at[mat][pl.ds(7 * r1, 7), dst, _rows(t, 128)] = _operands2(RHS, block, r1)
        return [functools.partial(task, t, r1) for t in range(NT // 4) for r1 in ORDER]

    def first_norm(fresh):
        for task in norm_tasks((top.at[0], xop.at[0]), 2, 0, 0, fresh):
            task(_now)

    def query_body(c, n, pacer, fresh):
        for j in range(n):
            nxt = c * n + j + 1
            if j == n - 1:
                nxt = jnp.minimum(nxt, NB - 1)
            pacer.add(norm_tasks((top.at[(j + 1) % n], xop.at[nxt]), 2, nxt, j % 2, fresh), 22)
            r = _rows(c * n + j, T)

            def emit(t, y):
                qa[t, r, :] = y * QSCALE
            matmul_a(top.at[j], WQ, emit, pacer)
        assert not pacer.todo

    def window_body(c):
        pacer = _Pacer(c)
        q_chunk = qa.at[:, _rows(c, CH)]
        x_chunk = xres.at[:, _rows(c, CH)]
        clear = {s: _bit_clear((WIN, 8, 128), 2, s) for s in (1, 2)}

        def project(mat, dst, j):
            def emit(t, y):
                dst[t, pl.ds(HALO + j * T, T), :] = y
                if j == 0:
                    first = jnp.broadcast_to(y[0:1], (HALO, 128))
                    dst[t, pl.ds(0, HALO), :] = jnp.where(c == 0, first, dst[t, pl.ds(CH, HALO), :])
            matmul_a(xop.at[2 * c + j], mat, emit, pacer)

        def pair_sum(x, s):
            return x + lax.select(clear[s], pltpu.roll(x, 128 - s, 2), pltpu.roll(x, s, 2))

        def logits(r, after):
            q = after(q_chunk[:, pl.ds(r, 8), :])
            x = jnp.stack([jnp.sum(q * ka[:, pl.ds(HALO + r - DIL * w, 8), :], axis=0) for w in range(WIN)])
            pa[:, pl.ds(r, 8), :] = pair_sum(x, 2)

        def softmax(r, after):
            x = pair_sum(after(pa[:, pl.ds(r, 8), :]), 1)
            if r < DIL * (WIN - 1):
                pos = c * CH + r + lax.broadcasted_iota(jnp.int32, x.shape, 1)
                x = jnp.where(pos >= DIL * lax.broadcasted_iota(jnp.int32, x.shape, 0), x, MASKED)
            e = jnp.exp2(x - jnp.max(x, axis=0, keepdims=True))
            pa[:, pl.ds(r, 8), :] = e * (1.0 / jnp.sum(e, axis=0, keepdims=True))

        def mix(j, r, after):
            r += j * T
            e = after(pa[:, pl.ds(r, 8), :])
            pa[:, pl.ds(r, 8), :] = functools.reduce(
                jnp.add, [e[w:w + 1] * va[:, pl.ds(HALO + r - DIL * w, 8), :] for w in range(WIN)])

        def project_out(j):
            def emit(t, y):
                x_chunk[t, _rows(j, T), :] = x_chunk[t, _rows(j, T), :] + y
            matmul_a(top.at[j], WO, emit, pacer)

        order = [r + dr for r in range(0, HT, 16) for dr in (0, 8, HT, HT + 8)]
        for j in range(2):
            pacer.add([functools.partial(logits, j * T + r) for r in order], 16, 28 * (j + 1))
            pacer.add([functools.partial(softmax, j * T + r) for r in order], 12, 28 * (j + 1) + 16)
            pacer.add(stage_tasks((top.at[j],), 2, pa.at[:, _rows(j, T)], functools.partial(mix, j)),
                      26, 28 * (j + 3))
            pacer.add([t for m in (WQ, WK, WV) for t in prep_b_tasks(m, 2 * c + j)], 26 - 2 * j, 140 * j)
        for mat, dst in ((WK, ka), (WV, va)):
            for j in range(2):
                project(mat, dst, j)
        for j in range(2):
            project_out(j)
        assert not pacer.todo

    def qkv_body(c):
        pacer = _Pacer(c)
        for j in range(2):
            i = 2 * c + j
            pacer.add(norm_tasks((bop.at[1 - j],), 4, jnp.minimum(i + 1, NCH - 1)), 250)
            for mat in (WQ, WV, WK):
                def emit(g, y):
                    if mat == WK:
                        kb[g, _rows(i, CH // 2), :] = _pack(y.astype(BF16))
                        return
                    y = (y * QSCALE if mat == WQ else y).astype(BF16)
                    for k in range(2):
                        (qtb if mat == WQ else vtb)[2 * i + k, _rows(g, 64), :] = _pack(y[k * T:(k + 1) * T].T)
                for _ in products_b(bop.at[j], mat, emit, pacer):
                    pass
        assert not pacer.todo

    def out_t(qb, a, head, n=1):
        return qa.at[qb * (QT // 2) + a // 2, _rows((a % 2) * (D // DH // n) + head, n * DH)]

    def attend(sbuf, i, pacer, do_pv, do_scores, between=None):
        on_vpu = [k * (S // KC) // NV for k in range(NV)]
        m_next = [None] * NU
        part = {}

        def keep(u, r, s):
            sbuf[u, pl.ds(r, s.shape[0]), :] = s
            m = jnp.max(s.reshape(-1, 8, QB), axis=0)
            m_next[u] = m if m_next[u] is None else jnp.maximum(m_next[u], m)

        def vpu_scores(u, r, d, after):
            k = after(kf[_rows(r, 8), :])
            q = jnp.broadcast_to(qf[u, :, :, pl.ds(d, 1), pl.ds(0, 128)], (QT, DH // 8, 8, 128))
            for j in range(DH // 8):
                c = u * DH + 8 * j + d
                term = q[:, j:j + 1] * jnp.broadcast_to(k[:, c:c + 1], (QT, 1, 8, 128))
                part[u] = term if d + j == 0 else part[u] + term
            if d == 7:
                keep(u, on_vpu[r // 2] * KC + (r % 2) * 8,
                     jnp.concatenate([part[u][a, 0] for a in range(QT)], axis=1))

        if do_scores:
            gn, qbn = (i + 1) & (NT - 1), (i + 1) >> 3
            qm = []
            for u in range(NU):
                qh = _unpack(qtb[_rows(qbn, QT), _rows(gn * NU + u, DH // 2), :])
                qf[u, :, :, :, pl.ds(0, 128)] = qh.astype(F32).reshape(QT, DH // 8, 8, 128)
                heads = [jnp.zeros((DH, QB), BF16)] * NU
                heads[u] = jnp.concatenate([qh[a] for a in range(QT)], axis=1)
                qm.append(jnp.concatenate(heads, axis=0))
            for j, c in enumerate(on_vpu):
                kf[_rows(j, 16), :] = _unpack(kb[gn, _rows(c * (KC // 16), 8), :]).astype(F32)
            pacer.add([functools.partial(vpu_scores, u, r, d)
                       for u in range(NU) for r in range(2 * NV) for d in range(8)],
                      NU * (S - 16 * NV) // 8, -12)
        for u in range(NU):
            if do_pv:
                head = (i & (NT - 1)) * NU + u
                v_rows = _rows(head, DH // 2)
                m = jnp.broadcast_to(jnp.max(mbuf[u], axis=0, keepdims=True), (8, QB))[None]
                l = None
            for c in range(S // KC):
                if do_pv:
                    sc = sbuf[u, _rows(c, KC), :].reshape(KC // 8, 8, QB)
                if do_scores:
                    pacer.overdue()
                    skip = 16 if c in on_vpu else 0
                    keys = _unpack(kb[gn, pl.ds((c * KC + skip) // 2, (KC - skip) // 2), :])
                    s = jnp.dot(keys, qm[u], preferred_element_type=F32)
                    keep(u, c * KC + skip, s)
                    for r in range(0, KC - skip, 8):
                        pacer.tick(s, r)
                if do_pv:
                    p = jnp.exp2(sc - m).reshape(KC, QB)
                    for r in reversed(range(0, KC, 8)):
                        l = p[r:r + 8] if l is None else l + p[r:r + 8]
                    pv = jnp.dot(_unpack(vtb[c, v_rows, :]), p.astype(BF16), preferred_element_type=F32)
                    acc = pv if c == 0 else abuf[u] + pv
                    if c + 1 < S // KC:
                        abuf[u] = acc
                if between is not None:
                    between()
            if do_pv:
                for a in range(QT):
                    lbuf[(i >> 3) * QT + a, _rows(head, 8), :] = l[:, a * 128:(a + 1) * 128]
                    out_t(i >> 3, a, head)[...] = acc[:, a * 128:(a + 1) * 128]
        if do_scores:
            assert not pacer.todo
            for u in range(NU):
                mbuf[u] = m_next[u]

    def out_stage_tasks(qb, j):
        def invert(a, after):
            l = [lbuf[qb * QT + 2 * j + a, pl.ds(k, D // DH, stride=8), :] for k in range(8)]
            linv[:, _rows(a, 128)] = 1.0 / after(functools.reduce(jnp.add, l))

        def normalise(a, g, after):
            inv = after(jnp.stack([jnp.broadcast_to(linv[pl.ds(NU * g + u, 1), _rows(a, 128)], (8, 128))
                                   for u in range(NU)]))
            o = out_t(qb, 2 * j + a, g, NU)[...].reshape(NU, DH // 8, 8, 128) * inv[:, None]
            xn[g, _rows(a, T), :] = o.reshape(128, 128).T
        return ([functools.partial(invert, a) for a in range(2)]
                + [functools.partial(normalise, a, g) for t in range(2) for g in range(t, NT, 2) for a in range(2)],
                stage_tasks((bop.at[j],), 4, xn, None))

    def out_products(qb, nxt, pacer):
        for j in range(2):
            first, second = out_stage_tasks(nxt, 0) if j else out_stage_tasks(qb, 1)
            pacer.add(first, 22)
            pacer.add(second, 74, 22)
            r = _rows(2 * qb + j, CH)

            def emit(t, y):
                x = xres[t, r, :] + y
                xres[t, r, :] = x
                xio[r, _rows(t, 128)] = x.astype(BF16)
            yield from products_b(bop.at[j], WO, emit, pacer)
        assert not pacer.todo

    def attention(rep, sbuf):
        steps = NQB * NT
        pacer = _Pacer(rep)
        pacer.add([t for i in range(W4 // 16) for t in prep_b_tasks(WO, i)], 230 * NU)
        attend(sbuf, -1, pacer, False, True)
        pl.loop(0, steps - 1)(lambda i: attend(sbuf, i, _Pacer(i), True, True))

        for tasks in out_stage_tasks(0, 0):
            for task in tasks:
                task(_now)
        out = out_products(0, 1, _Pacer(rep))
        count = [-16, 0]

        def between():
            count[0] += 1
            while count[1] * (NU * (S // KC) - 16) < count[0] * 190:
                next(out)
                count[1] += 1
        attend(sbuf, steps - 1, None, True, False, between)
        for _ in out:
            pass

    def copy(src, dst, idx, sem):
        return pltpu.make_async_copy(src.at[idx], dst.at[idx], sems.at[sem])

    def b_copy(c):
        return copy(wb_hbm, raw_b, (slice(None), _rows(c, W4 // NCH)), NCH + NQ + c)

    def bo_copy():
        return copy(wob_hbm, raw_ob, (slice(None),), 2 * NCH + NQ)

    def out_copy(c):
        return copy(xio, out_hbm, (_rows(c, QB),), c)

    def start_up(raw_a, raw_oa):
        step_rows = W2 // NCH

        def q_copy(i):
            return copy(wa_hbm, raw_a, (slice(None), _rows(i, W2 // NQ), pl.ds(0, D)), NCH + i)

        def o_tiles(i):
            return (i & 3, (i & 3) + 4)

        def step_copies(i, last):
            x_rows = pl.ds(_rows(2 * i + 1, T).start, T if last else 2 * T)
            return [copy(x_hbm, xio, (x_rows,), i),
                    copy(wa_hbm, raw_a, (slice(None), _rows(i, step_rows), pl.ds(D, 2 * D)), i)] + [
                copy(woa_hbm, raw_oa, (slice(None), i >> 2, slice(None), _rows(j, 128)), i) for j in o_tiles(i)]

        def start_step(i, last=False):
            for c in step_copies(i, last):
                c.start()
            if last:
                b_copy(0).start()

        def wait_step(i, last=False):
            for c in step_copies(i, last):
                c.wait()

        def prep_o(i, h4, h0, after):
            b = [[_swap_sublane_bits(
                [after(_pack(raw_oa[h4 * 4 + h, i >> 2, _rows(2 * h0 + d4, 16), _rows(j, 128)])) for h in range(4)])
                for j in o_tiles(i)] for d4 in range(2)]
            for d in range(4):
                rows = _rows(d * 8 + (i >> 2) * 4 + h0 * 2 + h4, 8)
                weight_a(WO, (i & 3) >> 1)[:, rows, _rows(i & 1, 128)] = _operands(
                    RHS, lambda k, j: _unpack(b[k][j][d]).astype(F32))

        x_first = copy(x_hbm, xio, (_rows(0, T),), NCH - 1)
        x_first.start()
        for i in range(NQ):
            q_copy(i).start()
        for i in range(AHEAD):
            start_step(i)
        for buf in (ka, va):
            buf[:, pl.ds(CH, HALO), :] = jnp.zeros((NT, HALO, 128), F32)
        x_first.wait()
        first_norm(True)

        @pl.loop(0, NQ)
        def _(i):
            q_copy(i).wait()
            prep_a(WQ, raw_a, i, W2 // NQ, _now)

        @pl.loop(0, NCH)
        def _(i):
            pl.when(i + AHEAD < NCH - 1)(lambda: start_step(i + AHEAD))
            pl.when(i + AHEAD == NCH - 1)(lambda: start_step(NCH - 1, True))
            pl.when(i < NCH - 1)(lambda: wait_step(i))
            pl.when(i == NCH - 1)(lambda: wait_step(NCH - 1, True))
            pacer = _Pacer(i)
            pacer.add([functools.partial(prep_a, m, raw_a, i * (step_rows // 16) + k, 16)
                       for k in range(step_rows // 16) for m in (WK, WV)], 30, 20)
            pacer.add([functools.partial(prep_o, i, k // 2, k % 2) for k in range(4)], 20, -1)
            pacer.overdue()
            query_body(i, 2, pacer, True)

    pl.run_scoped(start_up, pltpu.VMEM((2, W2, 3 * D), BF16), pltpu.VMEM((8, 2, 2 * DH, D), BF16))
    for c in range(1, NCH):
        b_copy(c).start()
    bo_copy().start()

    @pl.loop(0, 2)
    def _(rep):
        @pl.loop(0, NCH)
        def _(c):
            pl.when(rep == 0)(lambda: b_copy(c).wait())
            window_body(c)

        pl.when(rep == 0)(lambda: bo_copy().wait())
        for task in norm_tasks((bop.at[0],), 4, 0):
            task(_now)
        pl.loop(0, NCH // 2)(qkv_body)
        pl.run_scoped(functools.partial(attention, rep), pltpu.VMEM((NU, S, QB), F32))
        pl.when(rep == 1)(lambda: out_copy(0).start())

        @pl.loop(1, NQB)
        def _(c):
            for _ in out_products(c, jnp.minimum(c + 1, NQB - 1), _Pacer(c)):
                pass
            pl.when(rep == 1)(lambda: out_copy(c).start())

        @pl.when(rep == 0)
        def _():
            first_norm(False)
            pl.loop(0, NB // QS)(lambda c: query_body(c, QS, _Pacer(c), False))

    for c in range(NQB):
        out_copy(c).wait()


@jax.jit
def pallas_interleave_layers__sliding_local_dilated__softmax_full_mha__prompt_kernel(
    A_x: jax.Array,
    A_wqkv: jax.Array,
    A_wo: jax.Array,
    B_x: jax.Array,
    B_wqkv: jax.Array,
    B_wo: jax.Array,
):
    del B_x
    hbm = pl.BlockSpec(memory_space=pltpu.HBM)
    out = pl.pallas_call(
        _kernel,
        out_shape=jax.ShapeDtypeStruct((S, D), BF16),
        in_specs=[hbm] * 5,
        out_specs=hbm,
        scratch_shapes=[
            pltpu.VMEM((S, D), BF16),
            pltpu.VMEM((NT, S + 8, 128), F32),
            pltpu.VMEM((NB, 7, HT // 2, W2), U32),
            pltpu.VMEM((QS, 7, HT // 2, W2), U32),
            pltpu.VMEM((2, 49, HT // 2, W4), U32),
            pltpu.VMEM((NT, CH + 8, 128), F32),
            pltpu.VMEM((4, W4, 3 * D), BF16),
            pltpu.VMEM((4, W4, D), BF16),
            pltpu.VMEM((2, 7, W2 // 2, 256), U32),
            pltpu.VMEM((3, 2, 7, W2 // 2, 256), U32),
            pltpu.VMEM((4, 49, W4 // 2, W4), U32),
            pltpu.VMEM((NT, S + 8, 128), F32),
            pltpu.VMEM((NT, CH + 8, 128), F32),
            pltpu.VMEM((NT, HALO + CH + 8, 128), F32),
            pltpu.VMEM((NT, HALO + CH + 8, 128), F32),
            pltpu.VMEM((NT, S // 2, 128), U32),
            pltpu.VMEM((S // 128, D // 2, 128), U32),
            pltpu.VMEM((S // 128, D // 2, 128), U32),
            pltpu.VMEM((NU, 8, QB), F32),
            pltpu.VMEM((NU, DH, QB), F32),
            pltpu.VMEM((NB, D // DH * 8 + 8, 128), F32),
            pltpu.VMEM((D // DH, 256), F32),
            pltpu.VMEM((NU, QT, DH // 8, 8, 256), F32),
            pltpu.VMEM((16 * NV, 128), F32),
            pltpu.SemaphoreType.DMA((2 * NCH + NQ + 1,)),
        ],
        compiler_params=pltpu.CompilerParams(vmem_limit_bytes=127 * 2 ** 20),
        name="interleave_layers",
    )(A_x.reshape(S, D), A_wqkv.reshape(2, W2, 3 * D), A_wo.reshape(8, 2, 2 * DH, D),
      B_wqkv.reshape(4, W4, 3 * D), B_wo.reshape(4, W4, D))
    return out.reshape(1, S, D)
```

```python
import functools
import math

import jax
import jax.numpy as jnp
from jax import lax
import jax.experimental.pallas as pl
import jax.experimental.pallas.tpu as pltpu

S = 2048
D = 1024
DH = 32
WIN, DIL = 8, 2
HALO = 16
NT = D // 128
W2, W4 = D // 2, D // 4
HT = 64
T = 2 * HT
NB = S // T
CH = 2 * T
NCH = S // CH
QS = 4
NQ = 4
QB = 512
QT = QB // 128
NQB = S // QB
KC = 128
NU = 128 // DH
NV = 6
QSCALE = (DH ** -0.5) * math.log2(math.e)
MASKED = -1e9 * math.log2(math.e)
F32, BF16, U32 = jnp.float32, jnp.bfloat16, jnp.uint32
WQ, WK, WV, WO = range(4)

LHS = (((1, 0, 0), (1, 1, 1)), ((1, 1, 0), (1, 1, 1)), ((1, 0, 0),), ((1, 1, 1),),
       ((1, 0, 0), (1, 0, 1)), ((1, 1, 0), (-1, 0, 0)), ((1, 0, 1), (-1, 1, 1)))
RHS = (((1, 0, 0), (1, 1, 1)), ((1, 0, 0),), ((1, 0, 1), (-1, 1, 1)), ((1, 1, 0), (-1, 0, 0)),
       ((1, 1, 1),), ((1, 0, 0), (1, 0, 1)), ((1, 1, 0), (1, 1, 1)))
ORDER = (0, 3, 4, 6, 2, 1, 5)


def _combine(m):
    return ((m[0] + m[3] - m[4] + m[6], m[4] + m[2]), (m[3] + m[1], m[0] + m[2] - m[1] + m[5]))


def _signed_sum(terms, block):
    total = block(*terms[0][1:])
    for sign, i, j in terms[1:]:
        total = total + block(i, j) if sign > 0 else total - block(i, j)
    return total


def _operands(table, block):
    grid = {(i, j): block(i, j) for i in range(2) for j in range(2)}
    return _pack(jnp.stack([_signed_sum(terms, lambda i, j: grid[i, j]) for terms in table]).astype(BF16))


def _operands2(table, block, r):
    return _operands(table, lambda i, j: _signed_sum(table[r], lambda a, b: block(2 * a + i, 2 * b + j)))


def _pack(x):
    return pltpu.bitcast(x, U32)


def _unpack(x):
    return pltpu.bitcast(x, BF16)


def _now(x):
    return x


def _rows(i, n):
    return pl.ds(i * n if isinstance(i, int) else pl.multiple_of(i * n, n), n)


def _bit_clear(shape, axis, bit):
    return (lax.broadcasted_iota(jnp.int32, shape, axis) & bit) == 0


def _swap_lane_bits(tiles):
    last = tiles[0].ndim - 1
    t = [tiles[j] if j == 0 else pltpu.roll(tiles[j], 4 * j, last) for j in range(8)]
    t = [t[-f % 8] for f in range(8)]
    for b in range(3):
        clear = _bit_clear(t[0].shape, last, 4 << b)
        t = [lax.select(clear, t[f], t[(f - (1 << b)) % 8]) for f in range(8)]
    return [t[f] if f == 0 else pltpu.roll(t[f], 128 - 4 * f, last) for f in range(8)]


def _swap_sublane_bits(v):
    for bit, s in ((2, 4), (1, 2)):
        clear = _bit_clear((8, 128), 0, s)
        new = list(v)
        for r in range(4):
            if not r & bit:
                new[r] = lax.select(clear, v[r], pltpu.roll(v[r | bit], s, 0))
                new[r | bit] = lax.select(clear, pltpu.roll(v[r], 8 - s, 0), v[r | bit])
        v = new
    return v


class _Pacer:
    def __init__(self, index):
        self.never = index < 0
        self.masks = {}
        self.slot = 0
        self.todo = []

    def add(self, tasks, span, delay=0):
        for k, task in enumerate(tasks):
            self.todo.append((self.slot + delay + k * span // len(tasks), task))

    def _run(self, after):
        due = [t for s, t in self.todo if s < self.slot]
        self.todo = [(s, t) for s, t in self.todo if s >= self.slot]
        for task in due:
            task(after)

    def overdue(self):
        self._run(_now)

    def tick(self, result, row=0):
        seen = {}

        def after(x):
            if x.shape not in self.masks:
                self.masks[x.shape] = jnp.broadcast_to(self.never, x.shape)
            if (x.shape, x.dtype) not in seen:
                r = result[row:row + x.shape[-2], :128]
                r = r if x.dtype == F32 else pltpu.bitcast(r, x.dtype)
                seen[x.shape, x.dtype] = jnp.broadcast_to(r, x.shape)
            return lax.select(self.masks[x.shape], seen[x.shape, x.dtype], x)
        self.slot += 1
        self._run(after)


def _kernel(x_hbm, wa_hbm, woa_hbm, wb_hbm, wob_hbm, out_hbm,
            xio, xres, xop, top, bop, xn, raw_b, raw_ob, wq, wa, wb,
            qa, pa, ka, va, kb, qtb, vtb, mbuf, abuf, lbuf, linv, qf, kf, sems):

    def weight_a(mat, half):
        return wq.at[half] if mat == WQ else wa.at[mat - WK, half]

    def matmul_a(src, mat, emit, pacer):
        for n in range(NT // 2):
            m = {}
            for r in ORDER:
                m[r] = jnp.dot(_unpack(src[r]), _unpack(weight_a(mat, n >> 1)[r, :, _rows(n & 1, 128)]),
                               preferred_element_type=F32)
                pacer.tick(m[r])
            c = _combine(m)
            for j in range(2):
                emit(n + j * (NT // 2), jnp.concatenate([c[0][j], c[1][j]], axis=0))

    def products_b(src, mat, emit, pacer):
        for n in range(NT // 4):
            outer = {}
            for r1 in ORDER:
                m = {}
                for r2 in ORDER:
                    m[r2] = jnp.dot(_unpack(src[7 * r1 + r2]), _unpack(wb[mat, 7 * r1 + r2, :, _rows(n, 128)]),
                                    preferred_element_type=F32)
                    pacer.tick(m[r2])
                    yield
                outer[r1] = _combine(m)
            c = [[_combine({r: outer[r][i][j] for r in ORDER}) for j in range(2)] for i in range(2)]
            for j in range(4):
                emit(n + j * (NT // 4),
                     jnp.concatenate([c[i % 2][j % 2][i // 2][j // 2] for i in range(4)], axis=0))

    def stage_tasks(dsts, g, src, make_rows):
        def block(r, t, after):
            return lambda i, j: after(src[t + j * (NT // g), pl.ds(i * HT + r, 16), :])

        def store(k, r, t, ops):
            for dst in dsts:
                dst[pl.ds(k, 7), _rows(r // 16, 8), _rows(t, 128)] = ops

        def stage(r, after):
            for t in range(NT // g):
                store(0, r, t, _operands(LHS, block(r, t, after)))

        def stage2(r, t, r1, after):
            store(7 * r1, r, t, _operands2(LHS, block(r, t, after), r1))

        if make_rows is None:
            return [functools.partial(stage2, r, t, r1)
                    for r1 in ORDER for t in range(NT // g) for r in range(0, HT, 16)]
        tasks = []
        for r in range(0, HT + 16, 16):
            if r < HT:
                tasks += [functools.partial(make_rows, i * HT + r + dr) for i in range(g) for dr in (0, 8)]
            if r > 0 and g == 2:
                tasks.append(functools.partial(stage, r - 16))
            elif r > 0:
                tasks += [functools.partial(stage2, r - 16, t, r1) for t in range(NT // g) for r1 in ORDER]
        return tasks

    def norm_tasks(dsts, g, i, slot=0, fresh=False):
        x = xres.at[:, _rows(i, g * HT)]
        y = xn.at[:, _rows(slot, g * HT)]
        mean = {}

        def means(r0, after):
            for r in (r0, r0 + HT):
                if fresh:
                    v = xio.at[_rows(i, g * HT)][pl.ds(r, 16), :].astype(F32)
                    x[:, pl.ds(r, 16), :] = jnp.stack([v[:, t * 128:(t + 1) * 128] for t in range(NT)])
                for rr in (r, r + 8):
                    total = after(jnp.sum(x[:, pl.ds(rr, 8), :], axis=0))
                    mean[rr] = jnp.sum(total, axis=-1, keepdims=True) * (1.0 / D)

        def norm(r, after):
            c = x[:, pl.ds(r, 8), :] - after(jnp.broadcast_to(mean[r], (8, 128)))[None]
            var = jnp.sum(jnp.sum(c * c, axis=0), axis=-1, keepdims=True) * (1.0 / D)
            y[:, pl.ds(r, 8), :] = c * lax.rsqrt(var + 1e-5)[None]
        return ([functools.partial(means, k + r) for r in range(0, HT, 16) for k in range(0, g * HT, T)]
                + stage_tasks(dsts, g, y, norm))

    def prep_a(mat, raw, i, n, after):
        w = _swap_lane_bits([after(_pack(raw[:, _rows(i, n), _rows(mat * NT + j, 128)])) for j in range(NT)])
        for t in range(NT // 2):
            weight_a(mat, t >> 1)[:, _rows(i, n // 2), _rows(t & 1, 128)] = _operands(
                RHS, lambda k, j: _unpack(w[t + j * (NT // 2)][k]).astype(F32))

    def prep_b_tasks(mat, i):
        raw, tile0 = (raw_ob, 0) if mat == WO else (raw_b, mat * NT)
        src, dst = _rows(i, 16), _rows(i, 8)

        def task(t, r1, after):
            def block(k, j):
                return _unpack(after(_pack(raw[k, src, _rows(tile0 + t + j * (NT // 4), 128)]))).astype(F32)
            wb.at[mat][pl.ds(7 * r1, 7), dst, _rows(t, 128)] = _operands2(RHS, block, r1)
        return [functools.partial(task, t, r1) for t in range(NT // 4) for r1 in ORDER]

    def first_norm(fresh):
        for task in norm_tasks((top.at[0], xop.at[0]), 2, 0, 0, fresh):
            task(_now)

    def query_body(c, n, pacer, fresh):
        for j in range(n):
            nxt = c * n + j + 1
            if j == n - 1:
                nxt = jnp.minimum(nxt, NB - 1)
            pacer.add(norm_tasks((top.at[(j + 1) % n], xop.at[nxt]), 2, nxt, j % 2, fresh), 22)
            r = _rows(c * n + j, T)

            def emit(t, y):
                qa[t, r, :] = y * QSCALE
            matmul_a(top.at[j], WQ, emit, pacer)
        assert not pacer.todo

    def window_body(c):
        pacer = _Pacer(c)
        q_chunk = qa.at[:, _rows(c, CH)]
        x_chunk = xres.at[:, _rows(c, CH)]
        clear = {s: _bit_clear((WIN, 8, 128), 2, s) for s in (1, 2)}

        def project(mat, dst, j):
            def emit(t, y):
                dst[t, pl.ds(HALO + j * T, T), :] = y
                if j == 0:
                    first = jnp.broadcast_to(y[0:1], (HALO, 128))
                    dst[t, pl.ds(0, HALO), :] = jnp.where(c == 0, first, dst[t, pl.ds(CH, HALO), :])
            matmul_a(xop.at[2 * c + j], mat, emit, pacer)

        def pair_sum(x, s):
            return x + lax.select(clear[s], pltpu.roll(x, 128 - s, 2), pltpu.roll(x, s, 2))

        def logits(r, after):
            q = after(q_chunk[:, pl.ds(r, 8), :])
            x = jnp.stack([jnp.sum(q * ka[:, pl.ds(HALO + r - DIL * w, 8), :], axis=0) for w in range(WIN)])
            pa[:, pl.ds(r, 8), :] = pair_sum(x, 2)

        def softmax(r, after):
            x = pair_sum(after(pa[:, pl.ds(r, 8), :]), 1)
            if r < DIL * (WIN - 1):
                pos = c * CH + r + lax.broadcasted_iota(jnp.int32, x.shape, 1)
                x = jnp.where(pos >= DIL * lax.broadcasted_iota(jnp.int32, x.shape, 0), x, MASKED)
            e = jnp.exp2(x - jnp.max(x, axis=0, keepdims=True))
            pa[:, pl.ds(r, 8), :] = e * (1.0 / jnp.sum(e, axis=0, keepdims=True))

        def mix(j, r, after):
            r += j * T
            e = after(pa[:, pl.ds(r, 8), :])
            pa[:, pl.ds(r, 8), :] = functools.reduce(
                jnp.add, [e[w:w + 1] * va[:, pl.ds(HALO + r - DIL * w, 8), :] for w in range(WIN)])

        def project_out(j):
            def emit(t, y):
                x_chunk[t, _rows(j, T), :] = x_chunk[t, _rows(j, T), :] + y
            matmul_a(top.at[j], WO, emit, pacer)

        order = [r + dr for r in range(0, HT, 16) for dr in (0, 8, HT, HT + 8)]
        for j in range(2):
            pacer.add([functools.partial(logits, j * T + r) for r in order], 16, 28 * (j + 1))
            pacer.add([functools.partial(softmax, j * T + r) for r in order], 12, 28 * (j + 1) + 16)
            pacer.add(stage_tasks((top.at[j],), 2, pa.at[:, _rows(j, T)], functools.partial(mix, j)),
                      26, 28 * (j + 3))
            pacer.add([t for m in (WQ, WK, WV) for t in prep_b_tasks(m, 2 * c + j)], 26 - 2 * j, 140 * j)
        for mat, dst in ((WK, ka), (WV, va)):
            for j in range(2):
                project(mat, dst, j)
        for j in range(2):
            project_out(j)
        assert not pacer.todo

    def qkv_body(c):
        pacer = _Pacer(c)
        for j in range(2):
            i = 2 * c + j
            pacer.add(norm_tasks((bop.at[1 - j],), 4, jnp.minimum(i + 1, NCH - 1)), 250)
            for mat in (WQ, WV, WK):
                def emit(g, y):
                    if mat == WK:
                        kb[g, _rows(i, CH // 2), :] = _pack(y.astype(BF16))
                        return
                    y = (y * QSCALE if mat == WQ else y).astype(BF16)
                    for k in range(2):
                        (qtb if mat == WQ else vtb)[2 * i + k, _rows(g, 64), :] = _pack(y[k * T:(k + 1) * T].T)
                for _ in products_b(bop.at[j], mat, emit, pacer):
                    pass
        assert not pacer.todo

    def out_t(qb, a, head, n=1):
        return qa.at[qb * (QT // 2) + a // 2, _rows((a % 2) * (D // DH // n) + head, n * DH)]

    def attend(sbuf, i, pacer, do_pv, do_scores, between=None):
        on_vpu = [k * (S // KC) // NV for k in range(NV)]
        m_next = [None] * NU
        part = {}

        def keep(u, r, s):
            sbuf[u, pl.ds(r, s.shape[0]), :] = s
            m = jnp.max(s.reshape(-1, 8, QB), axis=0)
            m_next[u] = m if m_next[u] is None else jnp.maximum(m_next[u], m)

        def vpu_scores(u, r, d, after):
            k = after(kf[_rows(r, 8), :])
            q = jnp.broadcast_to(qf[u, :, :, pl.ds(d, 1), pl.ds(0, 128)], (QT, DH // 8, 8, 128))
            for j in range(DH // 8):
                c = u * DH + 8 * j + d
                term = q[:, j:j + 1] * jnp.broadcast_to(k[:, c:c + 1], (QT, 1, 8, 128))
                part[u] = term if d + j == 0 else part[u] + term
            if d == 7:
                keep(u, on_vpu[r // 2] * KC + (r % 2) * 8,
                     jnp.concatenate([part[u][a, 0] for a in range(QT)], axis=1))

        if do_scores:
            gn, qbn = (i + 1) & (NT - 1), (i + 1) >> 3
            qm = []
            for u in range(NU):
                qh = _unpack(qtb[_rows(qbn, QT), _rows(gn * NU + u, DH // 2), :])
                qf[u, :, :, :, pl.ds(0, 128)] = qh.astype(F32).reshape(QT, DH // 8, 8, 128)
                heads = [jnp.zeros((DH, QB), BF16)] * NU
                heads[u] = jnp.concatenate([qh[a] for a in range(QT)], axis=1)
                qm.append(jnp.concatenate(heads, axis=0))
            for j, c in enumerate(on_vpu):
                kf[_rows(j, 16), :] = _unpack(kb[gn, _rows(c * (KC // 16), 8), :]).astype(F32)
            pacer.add([functools.partial(vpu_scores, u, r, d)
                       for u in range(NU) for r in range(2 * NV) for d in range(8)],
                      NU * (S - 16 * NV) // 8, -12)
        for u in range(NU):
            if do_pv:
                head = (i & (NT - 1)) * NU + u
                v_rows = _rows(head, DH // 2)
                m = jnp.broadcast_to(jnp.max(mbuf[u], axis=0, keepdims=True), (8, QB))[None]
                l = None
            for c in range(S // KC):
                if do_pv:
                    sc = sbuf[u, _rows(c, KC), :].reshape(KC // 8, 8, QB)
                if do_scores:
                    pacer.overdue()
                    skip = 16 if c in on_vpu else 0
                    keys = _unpack(kb[gn, pl.ds((c * KC + skip) // 2, (KC - skip) // 2), :])
                    s = jnp.dot(keys, qm[u], preferred_element_type=F32)
                    keep(u, c * KC + skip, s)
                    for r in range(0, KC - skip, 8):
                        pacer.tick(s, r)
                if do_pv:
                    p = jnp.exp2(sc - m).reshape(KC, QB)
                    for r in reversed(range(0, KC, 8)):
                        l = p[r:r + 8] if l is None else l + p[r:r + 8]
                    pv = jnp.dot(_unpack(vtb[c, v_rows, :]), p.astype(BF16), preferred_element_type=F32)
                    acc = pv if c == 0 else abuf[u] + pv
                    if c + 1 < S // KC:
                        abuf[u] = acc
                if between is not None:
                    between()
            if do_pv:
                for a in range(QT):
                    lbuf[(i >> 3) * QT + a, _rows(head, 8), :] = l[:, a * 128:(a + 1) * 128]
                    out_t(i >> 3, a, head)[...] = acc[:, a * 128:(a + 1) * 128]
        if do_scores:
            assert not pacer.todo
            for u in range(NU):
                mbuf[u] = m_next[u]

    def out_stage_tasks(qb, j):
        def invert(a, after):
            l = [lbuf[qb * QT + 2 * j + a, pl.ds(k, D // DH, stride=8), :] for k in range(8)]
            linv[:, _rows(a, 128)] = 1.0 / after(functools.reduce(jnp.add, l))

        def normalise(a, g, after):
            inv = after(jnp.stack([jnp.broadcast_to(linv[pl.ds(NU * g + u, 1), _rows(a, 128)], (8, 128))
                                   for u in range(NU)]))
            o = out_t(qb, 2 * j + a, g, NU)[...].reshape(NU, DH // 8, 8, 128) * inv[:, None]
            xn[g, _rows(a, T), :] = o.reshape(128, 128).T
        return ([functools.partial(invert, a) for a in range(2)]
                + [functools.partial(normalise, a, g) for t in range(2) for g in range(t, NT, 2) for a in range(2)],
                stage_tasks((bop.at[j],), 4, xn, None))

    def out_products(qb, nxt, pacer):
        for j in range(2):
            first, second = out_stage_tasks(nxt, 0) if j else out_stage_tasks(qb, 1)
            pacer.add(first, 22)
            pacer.add(second, 74, 22)
            r = _rows(2 * qb + j, CH)

            def emit(t, y):
                x = xres[t, r, :] + y
                xres[t, r, :] = x
                xio[r, _rows(t, 128)] = x.astype(BF16)
            yield from products_b(bop.at[j], WO, emit, pacer)
        assert not pacer.todo

    def attention(rep, sbuf):
        steps = NQB * NT
        pacer = _Pacer(rep)
        pacer.add([t for i in range(W4 // 16) for t in prep_b_tasks(WO, i)], 230 * NU)
        attend(sbuf, -1, pacer, False, True)
        pl.loop(0, steps - 1)(lambda i: attend(sbuf, i, _Pacer(i), True, True))

        for tasks in out_stage_tasks(0, 0):
            for task in tasks:
                task(_now)
        out = out_products(0, 1, _Pacer(rep))
        count = [-16, 0]

        def between():
            count[0] += 1
            while count[1] * (NU * (S // KC) - 16) < count[0] * 190:
                next(out)
                count[1] += 1
        attend(sbuf, steps - 1, None, True, False, between)
        for _ in out:
            pass

    def copy(src, dst, idx, sem):
        return pltpu.make_async_copy(src.at[idx], dst.at[idx], sems.at[sem])

    def b_copy(c):
        return copy(wb_hbm, raw_b, (slice(None), _rows(c, W4 // NCH)), NCH + NQ + c)

    def bo_copy():
        return copy(wob_hbm, raw_ob, (slice(None),), 2 * NCH + NQ)

    def out_copy(c):
        return copy(xio, out_hbm, (_rows(c, QB),), c)

    def start_up(raw_a, raw_oa):
        step_rows = W2 // NCH

        def q_copy(i):
            return copy(wa_hbm, raw_a, (slice(None), _rows(i, W2 // NQ), pl.ds(0, D)), NCH + i)

        def o_tiles(i):
            return (i & 3, (i & 3) + 4)

        def step_copies(i, last):
            x_rows = pl.ds(_rows(2 * i + 1, T).start, T if last else 2 * T)
            return [copy(x_hbm, xio, (x_rows,), i),
                    copy(wa_hbm, raw_a, (slice(None), _rows(i, step_rows), pl.ds(D, 2 * D)), i)] + [
                copy(woa_hbm, raw_oa, (slice(None), i >> 2, slice(None), _rows(j, 128)), i) for j in o_tiles(i)]

        def wait_step(i, last=False):
            for c in step_copies(i, last):
                c.wait()

        def prep_o(i, h4, h0, after):
            b = [[_swap_sublane_bits(
                [after(_pack(raw_oa[h4 * 4 + h, i >> 2, _rows(2 * h0 + d4, 16), _rows(j, 128)])) for h in range(4)])
                for j in o_tiles(i)] for d4 in range(2)]
            for d in range(4):
                rows = _rows(d * 8 + (i >> 2) * 4 + h0 * 2 + h4, 8)
                weight_a(WO, (i & 3) >> 1)[:, rows, _rows(i & 1, 128)] = _operands(
                    RHS, lambda k, j: _unpack(b[k][j][d]).astype(F32))

        x_first = copy(x_hbm, xio, (_rows(0, T),), 2 * NCH + NQ + 1)
        x_first.start()
        for i in range(NQ):
            q_copy(i).start()
        for i in range(NCH):
            for c in step_copies(i, i == NCH - 1):
                c.start()
        b_copy(0).start()
        for buf in (ka, va):
            buf[:, pl.ds(CH, HALO), :] = jnp.zeros((NT, HALO, 128), F32)
        x_first.wait()
        first_norm(True)

        @pl.loop(0, NQ)
        def _(i):
            q_copy(i).wait()
            prep_a(WQ, raw_a, i, W2 // NQ, _now)

        @pl.loop(0, NCH)
        def _(i):
            pl.when(i < NCH - 1)(lambda: wait_step(i))
            pl.when(i == NCH - 1)(lambda: wait_step(NCH - 1, True))
            pacer = _Pacer(i)
            pacer.add([functools.partial(prep_a, m, raw_a, i * (step_rows // 16) + k, 16)
                       for k in range(step_rows // 16) for m in (WK, WV)], 30, 20)
            pacer.add([functools.partial(prep_o, i, k // 2, k % 2) for k in range(4)], 20, -1)
            pacer.overdue()
            query_body(i, 2, pacer, True)

    pl.run_scoped(start_up, pltpu.VMEM((2, W2, 3 * D), BF16), pltpu.VMEM((8, 2, 2 * DH, D), BF16))
    for c in range(1, NCH):
        b_copy(c).start()
    bo_copy().start()

    @pl.loop(0, 2)
    def _(rep):
        @pl.loop(0, NCH)
        def _(c):
            pl.when(rep == 0)(lambda: b_copy(c).wait())
            window_body(c)

        pl.when(rep == 0)(lambda: bo_copy().wait())
        for task in norm_tasks((bop.at[0],), 4, 0):
            task(_now)
        pl.loop(0, NCH // 2)(qkv_body)
        pl.run_scoped(functools.partial(attention, rep), pltpu.VMEM((NU, S, QB), F32))
        pl.when(rep == 1)(lambda: out_copy(0).start())

        @pl.loop(1, NQB)
        def _(c):
            for _ in out_products(c, jnp.minimum(c + 1, NQB - 1), _Pacer(c)):
                pass
            pl.when(rep == 1)(lambda: out_copy(c).start())

        @pl.when(rep == 0)
        def _():
            first_norm(False)
            pl.loop(0, NB // QS)(lambda c: query_body(c, QS, _Pacer(c), False))

    for c in range(NQB):
        out_copy(c).wait()


@jax.jit
def pallas_interleave_layers__sliding_local_dilated__softmax_full_mha__prompt_kernel(
    A_x: jax.Array,
    A_wqkv: jax.Array,
    A_wo: jax.Array,
    B_x: jax.Array,
    B_wqkv: jax.Array,
    B_wo: jax.Array,
):
    del B_x
    hbm = pl.BlockSpec(memory_space=pltpu.HBM)
    out = pl.pallas_call(
        _kernel,
        out_shape=jax.ShapeDtypeStruct((S, D), BF16),
        in_specs=[hbm] * 5,
        out_specs=hbm,
        scratch_shapes=[
            pltpu.VMEM((S, D), BF16),
            pltpu.VMEM((NT, S + 8, 128), F32),
            pltpu.VMEM((NB, 7, HT // 2, W2), U32),
            pltpu.VMEM((QS, 7, HT // 2, W2), U32),
            pltpu.VMEM((2, 49, HT // 2, W4), U32),
            pltpu.VMEM((NT, CH + 8, 128), F32),
            pltpu.VMEM((4, W4, 3 * D), BF16),
            pltpu.VMEM((4, W4, D), BF16),
            pltpu.VMEM((2, 7, W2 // 2, 256), U32),
            pltpu.VMEM((3, 2, 7, W2 // 2, 256), U32),
            pltpu.VMEM((4, 49, W4 // 2, W4), U32),
            pltpu.VMEM((NT, S + 8, 128), F32),
            pltpu.VMEM((NT, CH + 8, 128), F32),
            pltpu.VMEM((NT, HALO + CH + 8, 128), F32),
            pltpu.VMEM((NT, HALO + CH + 8, 128), F32),
            pltpu.VMEM((NT, S // 2, 128), U32),
            pltpu.VMEM((S // 128, D // 2, 128), U32),
            pltpu.VMEM((S // 128, D // 2, 128), U32),
            pltpu.VMEM((NU, 8, QB), F32),
            pltpu.VMEM((NU, DH, QB), F32),
            pltpu.VMEM((NB, D // DH * 8 + 8, 128), F32),
            pltpu.VMEM((D // DH, 256), F32),
            pltpu.VMEM((NU, QT, DH // 8, 8, 256), F32),
            pltpu.VMEM((16 * NV, 128), F32),
            pltpu.SemaphoreType.DMA((2 * NCH + NQ + 2,)),
        ],
        compiler_params=pltpu.CompilerParams(vmem_limit_bytes=127 * 2 ** 20),
        name="interleave_layers",
    )(A_x.reshape(S, D), A_wqkv.reshape(2, W2, 3 * D), A_wo.reshape(8, 2, 2 * DH, D),
      B_wqkv.reshape(4, W4, 3 * D), B_wo.reshape(4, W4, D))
    return out.reshape(1, S, D)
```
